```python
import jax
import jax.numpy as jnp

def _softmax(x, axis=-1):
    return jax.nn.softmax(x, axis=axis)

def _gelu(x):
    return jax.nn.gelu(x, approximate=True)

def _silu(x):
    return jax.nn.silu(x)

def _sigmoid(x):
    return jax.nn.sigmoid(x)

def _layernorm(x, axis=-1, eps=1e-05):
    m = jnp.mean(x, axis=axis, keepdims=True)
    v = jnp.var(x, axis=axis, keepdims=True)
    return (x - m) / jnp.sqrt(v + eps)

def _scatter_add(tgt, idx, src, axis=0):
    return tgt.at[idx].add(src)

def _segment_sum(src, seg, n):
    return jax.ops.segment_sum(src, seg, n)

class _Rng:

    def __init__(self, key):
        self._k = key

    def _next(self):
        self._k, sub = jax.random.split(self._k)
        return sub

    def normal(self, shape):
        return jax.random.normal(self._next(), shape, dtype=jnp.bfloat16)

    def randint(self, lo, hi, shape):
        return jax.random.randint(self._next(), shape, lo, hi, dtype=jnp.int32)

    def uniform(self, shape, lo=0.0, hi=1.0):
        return jax.random.uniform(self._next(), shape, jnp.bfloat16, lo, hi)

    def permutation(self, n):
        return jax.random.permutation(self._next(), n)
kernel_name = 'adaLN_cond__linear_kernel_hedgehog__moe_arch_mod__prompt'

def setup_inputs():
    _rng = _Rng(jax.random.key(int.from_bytes(__import__("os").urandom(4), "little")))
    _w = lambda a: (lambda t: t.astype(jnp.bfloat16) if jnp.issubdtype(t.dtype, jnp.floating) else t)(jnp.asarray(a))

    def _A_setup():
        B, S, D, H = (1, 2048, 1024, 32)
        Dh = D // H
        return {'x': _w((lambda *s: _rng.normal(s) * 0.05)(B, S, D)), 'wqkv': _w((lambda *s: _rng.normal(s) * 0.05)(D, 3 * D)), 'w_phi': _w((lambda *s: _rng.normal(s) * 0.05)(H, Dh, Dh) * Dh ** (-0.5)), 'wo': _w((lambda *s: _rng.normal(s) * 0.05)(D, D))}
    _A_in = _A_setup()

    def _B_setup():
        B, S, D, F, C = (1, 2048, 1024, 3584, 2)
        return {'x': _w((lambda *s: _rng.normal(s) * 0.05)(B, S, D)), 'w_r': _w((lambda *s: _rng.normal(s) * 0.05)(D)), 'w_gate': _w((lambda *s: _rng.normal(s) * 0.05)(D, F)), 'w_up': _w((lambda *s: _rng.normal(s) * 0.05)(D, F)), 'w_down': _w((lambda *s: _rng.normal(s) * 0.05)(F, D))}
    _B_in = _B_setup()
    return {'A_x': _A_in['x'], 'A_wqkv': _A_in['wqkv'], 'A_w_phi': _A_in['w_phi'], 'A_wo': _A_in['wo'], 'B_x': _B_in['x'], 'B_w_r': _B_in['w_r'], 'B_w_gate': _B_in['w_gate'], 'B_w_up': _B_in['w_up'], 'B_w_down': _B_in['w_down'], 'c': _w((lambda *s: _rng.normal(s) * 0.05)(1, 1024)), 'w_mod': _w((lambda *s: _rng.normal(s) * 0.05)(1024, 6 * 1024) * 1024 ** (-0.5))}

def reference(A_x, A_wqkv, A_w_phi, A_wo, B_x, B_w_r, B_w_gate, B_w_up, B_w_down, c, w_mod):

    def _A_ref(x, wqkv, w_phi, wo):
        B, S, D = x.shape
        H = 32
        Dh = D // H
        qkv = (lambda x, *d: x.transpose(*d))((x @ wqkv).reshape(B, S, 3, H, Dh), 2, 0, 3, 1, 4)
        q, k, v = (qkv[0], qkv[1], qkv[2])
        pq = jnp.einsum('bhsd,hdf->bhsf', q, w_phi)
        pk = jnp.einsum('bhsd,hdf->bhsf', k, w_phi)
        phi_q = jnp.concatenate([_softmax(pq, axis=-1), _softmax(-pq, axis=-1)], axis=-1)
        phi_k = jnp.concatenate([_softmax(pk, axis=-1), _softmax(-pk, axis=-1)], axis=-1)
        kv = jnp.einsum('bhsf,bhsd->bhfd', phi_k, v)
        z = jnp.einsum('bhsf->bhf', phi_k)
        num = jnp.einsum('bhqf,bhfd->bhqd', phi_q, kv)
        den = jnp.einsum('bhqf,bhf->bhq', phi_q, z)[..., None] + 1e-06
        o = num / den
        return (lambda x, *d: x.transpose(*d))(o, 0, 2, 1, 3).reshape(B, S, D) @ wo

    def _B_ref(x, w_r, w_gate, w_up, w_down):
        B, S, D = x.shape
        C = 2
        r = x @ w_r
        idx = jnp.argsort(-r, axis=-1)[:, :C]
        idx_e = jnp.repeat(idx.reshape(B, C, 1), D, axis=2)
        x_sel = jnp.take_along_axis(x, idx_e, axis=1)
        g = _silu(x_sel @ w_gate)
        u = x_sel @ w_up
        y = g * u @ w_down
        r_sel = _sigmoid(jnp.take_along_axis(r, idx, axis=1))
        y = y * r_sel.reshape(B, C, 1)
        b_off = (jnp.arange(B) * S).reshape(B, 1)
        flat_idx = (idx + b_off).reshape(B * C)
        zero = (x * 0.0).reshape(B * S, D)
        upd = _scatter_add(zero, flat_idx, y.reshape(B * C, D), axis=0)
        return x + upd.reshape(B, S, D)
    x = A_x
    mod = (_silu(c) @ w_mod).reshape(c.shape[0], 6, 1, -1)
    sa, ca, ga, sb, cb, gb = (mod[:, 0].copy(), mod[:, 1].copy(), mod[:, 2].copy(), mod[:, 3].copy(), mod[:, 4].copy(), mod[:, 5].copy())
    h = _layernorm(x, axis=-1) * (1 + ca) + sa
    x = x + ga * _A_ref(h, A_wqkv, A_w_phi, A_wo)
    h = _layernorm(x, axis=-1) * (1 + cb) + sb
    x = x + gb * _B_ref(h, B_w_r, B_w_gate, B_w_up, B_w_down)
    return x
```

```python
import functools
import math

import jax
import jax.numpy as jnp
from jax import lax
import jax.experimental.pallas as pl
import jax.experimental.pallas.tpu as pltpu

S, D, H, DH, F = 2048, 1024, 32, 32, 3584
PAIRS = H // 2
T = 256
NT_TILES = S // T
F_CHUNK = 512
LOG2E = math.log2(math.e)

F32 = jnp.float32
BF16 = jnp.bfloat16
U32 = jnp.uint32
I32 = jnp.int32

_NN = (((1,), (0,)), ((), ()))
_NT = (((1,), (1,)), ((), ()))
_TN = (((0,), (0,)), ((), ()))

(SEM_C, SEM_PHI, SEM_WR, SEM_MOD0, SEM_X0, SEM_WK, SEM_WV, SEM_X1, SEM_WQ,
 SEM_MOD1, SEM_WO, SEM_WG, SEM_WU, SEM_WD, SEM_FIX0, SEM_FIX1, NUM_SEMS) = range(17)


def _dot(a, b, dims):
    return lax.dot_general(a, b, dims, preferred_element_type=F32)


def _round_bf16(x):
    return x.astype(BF16).astype(F32)


def _to_words(x):
    return pltpu.bitcast(x.astype(BF16), U32)


def _from_words(w):
    return pltpu.bitcast(w, BF16)


def _iota(shape, axis):
    return lax.broadcasted_iota(I32, shape, axis)


def _layernorm_mod(x, scale1p, shift):
    rows = x.shape[0]
    mean = jnp.sum(x, axis=-1, keepdims=True) * (1.0 / D)
    xc = x - mean
    var = jnp.sum(xc * xc, axis=-1, keepdims=True) * (1.0 / D)
    std = _round_bf16(jnp.sqrt(_round_bf16(_round_bf16(var) + 1e-5)))
    y = (xc * (1.0 / std)).reshape(rows // 8, 8, D)
    return (y * scale1p[None] + shift[None]).reshape(rows, D)


def _head_allreduce(x, op):
    r = x[0]
    for i in range(1, x.shape[0]):
        r = op(r, x[i])
    r = op(r, pltpu.roll(r, 4, 0))
    return op(r, pltpu.roll(r, 2, 0))


def _feature_map(p):
    p = p.reshape(8, 8, p.shape[-1])
    hi = _head_allreduce(p, jnp.maximum)
    lo = _head_allreduce(p, jnp.minimum)
    e_pos = jnp.exp2(p - hi[None])
    e_neg = jnp.exp2(lo[None] - p)
    inv_pos = 1.0 / _head_allreduce(e_pos, jnp.add)
    inv_neg = 1.0 / _head_allreduce(e_neg, jnp.add)
    return e_pos * inv_pos[None], e_neg * inv_neg[None]


def _kernel(x_hbm, wqkv_hbm, wphi_hbm, wo_hbm, wr_hbm, wg_hbm, wu_hbm, wd_hbm, c_hbm, wmod_hbm,
            out_hbm,
            x_v, wqkv_v, wphi_v, wo_v, wr_v, wg_v, wu_v, wd_v, c_v, wmod_v,
            wqT, wkT, wvT, h_v, x1_v, out_v, mod_v, kv_acc, z_acc, kvT, top_v,
            sems, out_sems):

    def cols(ref, start, size):
        return ref.at[:, pl.ds(start, size)]

    def rows(ref, start, size):
        return ref.at[pl.ds(start, size), :]

    def copy(src, dst, sem):
        return pltpu.make_async_copy(src, dst, sems.at[sem])

    cp_c = copy(c_hbm, c_v, SEM_C)
    cp_phi = copy(wphi_hbm, wphi_v, SEM_PHI)
    cp_wr = copy(wr_hbm, wr_v, SEM_WR)
    cp_wk = copy(cols(wqkv_hbm, D, D), cols(wqkv_v, D, D), SEM_WK)
    cp_mod0 = copy(cols(wmod_hbm, 0, 2 * D), cols(wmod_v, 0, 2 * D), SEM_MOD0)
    cp_x0 = copy(rows(x_hbm, 0, T), rows(x_v, 0, T), SEM_X0)
    cp_wv = copy(cols(wqkv_hbm, 2 * D, D), cols(wqkv_v, 2 * D, D), SEM_WV)
    cp_x1 = copy(rows(x_hbm, T, S - T), rows(x_v, T, S - T), SEM_X1)
    cp_wq = copy(cols(wqkv_hbm, 0, D), cols(wqkv_v, 0, D), SEM_WQ)
    cp_mod1 = copy(cols(wmod_hbm, 2 * D, 4 * D), cols(wmod_v, 2 * D, 4 * D), SEM_MOD1)
    cp_wo = copy(wo_hbm, wo_v, SEM_WO)
    cp_wg = copy(wg_hbm, wg_v, SEM_WG)
    cp_wu = copy(wu_hbm, wu_v, SEM_WU)
    cp_wd = copy(wd_hbm, wd_v, SEM_WD)
    for cp in (cp_c, cp_phi, cp_wk, cp_mod0, cp_x0, cp_wv, cp_x1, cp_wr, cp_wq, cp_mod1,
               cp_wo, cp_wg, cp_wu, cp_wd):
        cp.start()

    def fold_phi(col0, dst):
        row = _iota((128, DH), 0)
        select = ((row % 64) // 2 == _iota((128, DH), 1)).astype(BF16)
        row = _iota((128, 128), 0)
        same_head = (row // 64) * 2 + row % 2 == _iota((128, 128), 1) // DH
        for g in range(D // 128):
            phi = wphi_v[g * 128:(g + 1) * 128, :]
            bd = jnp.where(same_head, _dot(select, phi, _NT), 0.0).astype(BF16)
            w = wqkv_v[:, col0 + g * 128:col0 + (g + 1) * 128]
            dst[g * 64:(g + 1) * 64, :] = _to_words(_dot(bd, w, _NT) * LOG2E)

    cp_phi.wait()
    cp_wk.wait()
    fold_phi(D, wkT)

    cp_c.wait()
    c = c_v[...].astype(F32)
    silu_c = jnp.broadcast_to(c * jax.nn.sigmoid(c), (16, D)).astype(BF16)

    def modulation(i, plus_one=False):
        m = _round_bf16(_dot(silu_c, wmod_v[:, i * D:(i + 1) * D], _NN)[:8])
        mod_v[i] = _round_bf16(1.0 + m) if plus_one else m

    cp_mod0.wait()
    modulation(0)
    modulation(1, plus_one=True)

    cp_wv.wait()
    for g in range(D // 128):
        w = wqkv_v[:, 2 * D + g * 128:2 * D + (g + 1) * 128].astype(F32)
        wvT[g * 64:(g + 1) * 64, :] = _to_words(w.T)

    kv_acc[...] = jnp.zeros_like(kv_acc)
    z_acc[...] = jnp.zeros_like(z_acc)
    cp_x0.wait()
    cp_x1.wait()

    def key_value_tile(i, carry):
        r0 = pl.multiple_of(i * T, T)
        h = _layernorm_mod(x_v[pl.ds(r0, T), :].astype(F32), mod_v[1], mod_v[0]).astype(BF16)
        h_v[pl.ds(pl.multiple_of(i * (T // 2), T // 2), T // 2), :] = pltpu.bitcast(h, U32)
        for g in range(D // 128):
            pk = _dot(_from_words(wkT[g * 64:(g + 1) * 64, :]), h, _NT)
            v = _dot(_from_words(wvT[g * 64:(g + 1) * 64, :]), h, _NT).astype(BF16)
            for j in range(2):
                pair = 2 * g + j
                pos, neg = _feature_map(pk[j * 64:(j + 1) * 64])
                phi = jnp.concatenate([pos, neg], axis=0).reshape(128, T)
                zs = phi[:, :128]
                for l in range(1, T // 128):
                    zs = zs + phi[:, l * 128:(l + 1) * 128]
                z_acc[pair] += zs
                kv_acc[pair] += _dot(v[j * 64:(j + 1) * 64], phi.astype(BF16), _NT)
        return carry

    lax.fori_loop(0, NT_TILES, key_value_tile, 0)

    same_head = _iota((64, 128), 0) // DH == _iota((64, 128), 1) % 2
    for pair in range(PAIRS):
        kvT[pair] = _to_words(jnp.where(same_head, kv_acc[pair], 0.0))
        z_acc[pair] = jnp.broadcast_to(jnp.sum(z_acc[pair], axis=-1, keepdims=True), (128, 128))

    cp_wq.wait()
    fold_phi(0, wqT)
    cp_mod1.wait()
    modulation(2)
    modulation(3)
    modulation(4, plus_one=True)
    modulation(5)
    cp_wo.wait()
    cp_wr.wait()
    wr = wr_v[...].astype(F32)
    for l in range(D // 128):
        mod_v[6, :, l * 128:(l + 1) * 128] = jnp.broadcast_to(wr[l:l + 1, :], (8, 128))

    def out_copy(i):
        r0 = pl.multiple_of(i * T, T)
        return pltpu.make_async_copy(rows(out_v, r0, T), rows(out_hbm, r0, T), out_sems.at[i])

    def query_tile(i, top):
        r0 = pl.multiple_of(i * T, T)
        h = _from_words(h_v[pl.ds(pl.multiple_of(i * (T // 2), T // 2), T // 2), :])
        even = _iota((8, T), 0) % 2 == 0
        o_blocks = []
        for g in range(D // 128):
            pq = _dot(_from_words(wqT[g * 64:(g + 1) * 64, :]), h, _NT)
            for j in range(2):
                pair = 2 * g + j
                pos, neg = _feature_map(pq[j * 64:(j + 1) * 64])
                phi = jnp.concatenate([pos, neg], axis=0)
                z = jnp.concatenate([z_acc[pair]] * (T // 128), axis=1).reshape(16, 8, T)
                inv = 1.0 / (_head_allreduce(phi * z, jnp.add) + 1e-6)
                swapped = pltpu.roll(inv, 1, 0)
                inv0 = jnp.where(even, inv, swapped)
                inv1 = jnp.where(even, swapped, inv)
                num = _dot(_from_words(kvT[pair]), phi.reshape(128, T).astype(BF16), _NN)
                num = num.reshape(8, 8, T)
                o = jnp.concatenate([num[:4] * inv0[None], num[4:] * inv1[None]], axis=0)
                o_blocks.append(o.reshape(64, T).astype(BF16))
        attn = _dot(jnp.concatenate(o_blocks, axis=0), wo_v[...], _TN)
        x = x_v[pl.ds(r0, T), :].astype(F32)
        x1 = (x.reshape(T // 8, 8, D) + mod_v[2][None] * attn.reshape(T // 8, 8, D)).reshape(T, D)
        x1_v[pl.ds(r0, T), :] = x1
        h2 = _layernorm_mod(x1, mod_v[4], mod_v[3]).reshape(T // 8, 8, D)
        out = x1.reshape(T // 8, 8, D) + mod_v[5][None] * h2
        out_v[pl.ds(r0, T), :] = out.reshape(T, D).astype(BF16)
        out_copy(i).start()

        score = _round_bf16(jnp.sum(h2 * mod_v[6][None], axis=-1, keepdims=True))
        best, best_i, second, second_i = top
        token = r0 + _iota((8, 1), 0)
        for b in range(T // 8):
            s, t = score[b], token + 8 * b
            above_best, above_second = s > best, s > second
            second = jnp.where(above_best, best, jnp.where(above_second, s, second))
            second_i = jnp.where(above_best, best_i, jnp.where(above_second, t, second_i))
            best = jnp.where(above_best, s, best)
            best_i = jnp.where(above_best, t, best_i)
        return best, best_i, second, second_i

    lowest = jnp.full((8, 1), -jnp.inf, F32)
    zero_i = jnp.zeros((8, 1), I32)
    best, best_i, second, second_i = lax.fori_loop(
        0, NT_TILES, query_tile, (lowest, zero_i, lowest, zero_i))

    scores = jnp.concatenate([best, second], axis=0)
    tokens = jnp.concatenate([best_i, second_i], axis=0)

    def take_top(scores):
        top = jnp.max(scores, axis=0, keepdims=True)
        tok = jnp.min(jnp.where(scores == top, tokens, S - 1).astype(F32), axis=0, keepdims=True)
        return top, tok.astype(I32)

    score0, tok0 = take_top(scores)
    score1, tok1 = take_top(jnp.where(tokens == tok0, -jnp.inf, scores))
    idx = [jnp.clip(tok0[0, 0], 0, S - 1), jnp.clip(tok1[0, 0], 0, S - 1)]
    base = [pl.multiple_of((t // 16) * 16, 16) for t in idx]

    row16 = _iota((16, D), 0)
    x1_blk, h2_blk = [], []
    h_sel = jnp.zeros((16, D), F32)
    for k in range(2):
        x1 = x1_v[pl.ds(base[k], 16), :]
        h2 = _layernorm_mod(x1, mod_v[4], mod_v[3])
        picked = jnp.sum(jnp.where(row16 == idx[k] % 16, h2, 0.0), axis=0, keepdims=True)
        h_sel = jnp.where(row16 == k, picked, h_sel)
        x1_blk.append(x1)
        h2_blk.append(h2)
    h_sel = h_sel.astype(BF16)

    cp_wg.wait()
    cp_wu.wait()
    cp_wd.wait()
    y = jnp.zeros((16, D), F32)
    for f in range(F // F_CHUNK):
        sl = slice(f * F_CHUNK, (f + 1) * F_CHUNK)
        gate = _dot(h_sel, wg_v[:, sl], _NN)
        up = _dot(h_sel, wu_v[:, sl], _NN)
        act = (gate * jax.nn.sigmoid(gate) * up).astype(BF16)
        y = y + _dot(act, wd_v[sl, :], _NN)
    y_sel = [y[0:1] * jax.nn.sigmoid(score0), y[1:2] * jax.nn.sigmoid(score1)]

    for i in range(NT_TILES):
        out_copy(i).wait()

    gb = jnp.concatenate([mod_v[5], mod_v[5]], axis=0)
    for k in range(2):
        upd = jnp.zeros((16, D), F32)
        for m in range(2):
            upd = jnp.where(row16 == idx[m] - base[k], y_sel[m], upd)
        out_v[pl.ds(base[k], 16), :] = (x1_blk[k] + gb * (h2_blk[k] + upd)).astype(BF16)

    fix0 = copy(rows(out_v, base[0], 16), rows(out_hbm, base[0], 16), SEM_FIX0)
    fix1 = copy(rows(out_v, base[1], 16), rows(out_hbm, base[1], 16), SEM_FIX1)
    fix0.start()

    @pl.when(base[0] != base[1])
    def _():
        fix1.start()
        fix1.wait()

    fix0.wait()


@jax.jit
def pallas_adaLN_cond__linear_kernel_hedgehog__moe_arch_mod__prompt_kernel(
    A_x: jax.Array,
    A_wqkv: jax.Array,
    A_w_phi: jax.Array,
    A_wo: jax.Array,
    B_x: jax.Array,
    B_w_r: jax.Array,
    B_w_gate: jax.Array,
    B_w_up: jax.Array,
    B_w_down: jax.Array,
    c: jax.Array,
    w_mod: jax.Array,
):
    del B_x
    out = pl.pallas_call(
        _kernel,
        out_shape=jax.ShapeDtypeStruct((S, D), BF16),
        in_specs=[pl.BlockSpec(memory_space=pl.ANY)] * 10,
        out_specs=pl.BlockSpec(memory_space=pl.ANY),
        scratch_shapes=[
            pltpu.VMEM((S, D), BF16),
            pltpu.VMEM((D, 3 * D), BF16),
            pltpu.VMEM((H * DH, DH), BF16),
            pltpu.VMEM((D, D), BF16),
            pltpu.VMEM((D // 128, 128), BF16),
            pltpu.VMEM((D, F), BF16),
            pltpu.VMEM((D, F), BF16),
            pltpu.VMEM((F, D), BF16),
            pltpu.VMEM((1, D), BF16),
            pltpu.VMEM((D, 6 * D), BF16),
            pltpu.VMEM((D // 2, D), U32),
            pltpu.VMEM((D // 2, D), U32),
            pltpu.VMEM((D // 2, D), U32),
            pltpu.VMEM((S // 2, D), U32),
            pltpu.VMEM((S, D), F32),
            pltpu.VMEM((S, D), BF16),
            pltpu.VMEM((7, 8, D), F32),
            pltpu.VMEM((PAIRS, 64, 128), F32),
            pltpu.VMEM((PAIRS, 128, 128), F32),
            pltpu.VMEM((PAIRS, 32, 128), U32),
            pltpu.VMEM((8, 128), F32),
            pltpu.SemaphoreType.DMA((NUM_SEMS,)),
            pltpu.SemaphoreType.DMA((NT_TILES,)),
        ],
        compiler_params=pltpu.CompilerParams(vmem_limit_bytes=110 * 1024 * 1024),
        name="hedgehog_moe",
    )(
        A_x.reshape(S, D), A_wqkv, A_w_phi.reshape(H * DH, DH), A_wo,
        B_w_r.reshape(D // 128, 128), B_w_gate, B_w_up, B_w_down, c, w_mod,
    )
    return out.reshape(1, S, D)
```

```python
import functools
import itertools
import math


import jax
import jax.numpy as jnp
from jax import lax
import jax.experimental.pallas as pl
import jax.experimental.pallas.tpu as pltpu

S, D, H, DH, F = 2048, 1024, 32, 32, 3584
PAIRS = H // 2
T = 256
TILES = S // T
SG = 4
UNITS = TILES * SG
HALF = D // 2
F_CHUNK = 512
MOD_CHUNK = 256
LOG2E = math.log2(math.e)
NOPS = 7

KEY_SLOTS = (2, 3, 5, 6)
QUERY_SLOTS = (2, 3, 4, 5)
LN_SLOTS = (1, 3, 4, 6)
STORE_SLOT = 6
FINISH_SLOTS = ((1, 3), (2, 4), (5, 7), (6, 8))
FOLD_Q_UNIT = min(12, UNITS - 8)
MOD_UNIT = min(20, UNITS - 4)
LAST_ROWS = 64

F32 = jnp.float32
BF16 = jnp.bfloat16
U32 = jnp.uint32
I32 = jnp.int32

_NN = (((1,), (0,)), ((), ()))
_NT = (((1,), (1,)), ((), ()))


def _dot(a, b, dims):
    return lax.dot_general(a, b, dims, preferred_element_type=F32)


def _round_bf16(x):
    return x.astype(BF16).astype(F32)


def _bits(x):
    return pltpu.bitcast(x, U32)


def _iota(shape, axis):
    return lax.broadcasted_iota(I32, shape, axis)


def _recip(x):
    return pl.reciprocal(x, full_range=False)


def _join(tokens):
    return functools.reduce(jnp.bitwise_or, tokens)


def _left_operands(a11, a12, a21, a22):
    return a11 + a22, a21 + a22, a11, a22, a11 + a12, a21 - a11, a12 - a22


def _right_operands(b11, b12, b21, b22):
    return b11 + b22, b11, b12 - b22, b21 - b11, b22, b11 + b12, b21 + b22


def _row_sum(x):
    return jnp.sum(x, axis=-1, keepdims=True)


def _inv_std(centered):
    return lax.rsqrt(_row_sum(centered * centered) * (1.0 / D) + 1e-5)


def _row_token(x):
    return _join([_bits(jnp.broadcast_to(x[i], (8, 128))) for i in range(x.shape[0])])


def _pack_rows(x):
    x = x.reshape(x.shape[0] // 16, 2, 8, x.shape[1])
    words = pltpu.pack_elementwise([x[:, 0], x[:, 1]], packed_dtype=BF16)
    return words.reshape(words.shape[0] * 8, words.shape[2])


def _head_allreduce(x, op):
    r = x[0]
    for i in range(1, x.shape[0]):
        r = op(r, x[i])
    r = op(r, pltpu.roll(r, 4, 0))
    return op(r, pltpu.roll(r, 2, 0))


def _feature_map(p):
    p = p.reshape(8, 8, 128)
    e_pos = jnp.exp2(p - _head_allreduce(p, jnp.maximum)[None])
    e_neg = jnp.exp2(_head_allreduce(p, jnp.minimum)[None] - p)
    inv_pos = _recip(_head_allreduce(e_pos, jnp.add))
    inv_neg = _recip(_head_allreduce(e_neg, jnp.add))
    phi = jnp.concatenate([e_pos * inv_pos[None], e_neg * inv_neg[None]], axis=0)
    return phi.reshape(128, 128), _bits(inv_pos) | _bits(inv_neg)


def _kernel(x_hbm, wqkv_hbm, wphi_hbm, wo_hbm, wr_hbm, wg_hbm, wu_hbm, wd_hbm, c_hbm, wmod_hbm,
            out_hbm,
            x_v, wqkv_v, wphi_v, wo_v, wr_v, wg_v, wu_v, wd_v, c_v, wmod_v,
            wq_s, wk_s, wv_s, wo_s, picked_v, out_v, mod_a, mod_b, kv_acc, z_acc,
            sems, *x1_v):
    sem_ids = itertools.count()

    def copy(src, dst):
        return pltpu.make_async_copy(src, dst, sems.at[next(sem_ids)])

    def copy_cols(src, dst, start, size):
        return copy(src.at[:, pl.ds(start, size)], dst.at[:, pl.ds(start, size)])

    def copy_blocks(src, dst, start, size):
        return copy(src.at[pl.ds(start, size)], dst.at[pl.ds(start, size)])

    cp_c, cp_phi, cp_wr = copy(c_hbm, c_v), copy(wphi_hbm, wphi_v), copy(wr_hbm, wr_v)
    cp_x = [copy_blocks(x_hbm, x_v, 16 * i, 16) for i in range(3)]
    cp_x.append(copy_blocks(x_hbm, x_v, 48, S // 16 - 48))
    cp_mod_a = [copy_cols(wmod_hbm, wmod_v, c0, MOD_CHUNK) for c0 in range(0, 2 * D, MOD_CHUNK)]
    cp_wk = [copy_cols(wqkv_hbm, wqkv_v, D + 256 * sg, 256) for sg in range(SG)]
    cp_wv = [copy_cols(wqkv_hbm, wqkv_v, 2 * D + 256 * sg, 256) for sg in range(SG)]
    cp_wq = copy_cols(wqkv_hbm, wqkv_v, 0, D)
    cp_mod_b = copy_cols(wmod_hbm, wmod_v, 2 * D, 4 * D)
    cp_wo = copy_blocks(wo_hbm, wo_v, 0, SG)
    cp_ffn = [copy(wg_hbm, wg_v), copy(wu_hbm, wu_v), copy(wd_hbm, wd_v)]
    cp_out = [copy_blocks(out_v, out_hbm, 16 * i, 16) for i in range(TILES)]
    for cp in (cp_c, cp_x[0], cp_phi, *cp_mod_a, cp_wk[0], cp_wv[0], cp_wk[1], cp_wv[1], cp_x[1],
               cp_wk[2], cp_wv[2], cp_wk[3], cp_wv[3], cp_x[2], cp_x[3], cp_wr, cp_wq, cp_mod_b,
               cp_wo, *cp_ffn):
        cp.start()

    cp_c.wait()
    c = c_v[...].astype(F32)
    silu_c = jnp.broadcast_to(c * jax.nn.sigmoid(c), (16, D)).astype(BF16)
    never = jnp.broadcast_to(c[:, :128] * c[:, :128], (8, 128)) < 0.0
    zero = jnp.max(never.astype(F32)).astype(I32)
    stamps = itertools.count(1)

    def at(i):
        return i + zero * next(stamps)

    def after(words, token):
        head = jnp.where(never, token, words[:8, :128])
        if words.shape[1] > 128:
            head = jnp.concatenate([head, words[:8, 128:]], axis=1)
        return jnp.concatenate([head, words[8:]], axis=0)

    def block_product(left, right, dims, tasks):
        def m(n, slot):
            tokens = [fn() for at_slot, fn in tasks if at_slot == slot]
            tokens = [t for t in tokens if t is not None]
            operands = [left(n), right(n)]
            for k, op in enumerate(operands):
                if op.dtype == U32:
                    operands[k] = pltpu.bitcast(after(op, _join(tokens)) if tokens else op, BF16)
            return _dot(*operands, dims)

        m1, m2 = m(0, 0), m(1, 1)
        c22 = m1 - m2
        m4 = m(3, 2)
        c21 = m2 + m4
        c11 = m1 + m4
        m3 = m(2, 3)
        c22 = c22 + m3
        m5 = m(4, 4)
        c12 = m3 + m5
        c11 = c11 - m5 + m(6, 5)
        c22 = c22 + m(5, 6)
        return c11, c12, c21, c22

    def modulation(col0):
        i, c0 = divmod(col0, D)
        m = _round_bf16(_dot(silu_c, wmod_v[:, col0:col0 + MOD_CHUNK], _NN)[:8])
        dst, row = (mod_a, i) if i < 2 else (mod_b, i - 2)
        dst[row, :, c0:c0 + MOD_CHUNK] = _round_bf16(1.0 + m) if i % 3 == 1 else m

    def phi_blocks():
        def packed_row(shape):
            r = _iota(shape, 0)
            return r // 16 * 16 + r % 8 * 2 + r // 8 % 2

        select = ((packed_row((128, DH)) % 64) // 2 == _iota((128, DH), 1)).astype(BF16)
        row = packed_row((128, 128))
        same_head = (row // 64) * 2 + row % 2 == _iota((128, 128), 1) // DH
        return [jnp.where(same_head, _dot(select, wphi_v[g * 128:(g + 1) * 128, :], _NT), 0.0)
                .astype(BF16) for g in range(D // 128)]

    def fold_phi(col0, dst, sg, l):
        quads = []
        for g in (2 * sg, 2 * sg + 1):
            cs = slice(col0 + g * 128, col0 + (g + 1) * 128)
            w = jnp.concatenate([wqkv_v[r:r + 128, cs] for r in (l * 128, HALF + l * 128)], axis=0)
            folded = _dot(phi_bd[g], w, _NT) * LOG2E
            quads += [folded[:, :128], folded[:, 128:]]
        for n, op in enumerate(_left_operands(*quads)):
            dst[sg * NOPS + n, :, l * 128:(l + 1) * 128] = _pack_rows(op)

    def transpose_wv(sg):
        w = wqkv_v[:, 2 * D + sg * 256:2 * D + (sg + 1) * 256].astype(F32)
        ops = _left_operands(w[:HALF, :128], w[HALF:, :128], w[:HALF, 128:], w[HALF:, 128:])
        for n, op in enumerate(ops):
            wv_s[sg * NOPS + n] = _bits(op.astype(BF16).T)

    def split_wo(cp, sg, token):
        wo_v[SG, :16, :128] = pltpu.bitcast(token, BF16)
        words = _bits(wo_v[at(sg), :, cp * 256:(cp + 1) * 256])
        halves = []
        for e in range(2):
            w = pltpu.unpack_elementwise(words, index=e, packed_dtype=BF16, unpacked_dtype=F32)
            halves.append(_right_operands(w[:64, :128], w[:64, 128:], w[64:, :128], w[64:, 128:]))
        for n in range(NOPS):
            wo_s[cp * NOPS + n, sg * 64:(sg + 1) * 64, :] = pltpu.pack_elementwise(
                [halves[0][n], halves[1][n]], packed_dtype=BF16)

    stats, h_parts, h_ops = {}, {}, {}

    def load_rows(i, b):
        return jnp.concatenate([x_v[at(i * 16 + half * 8 + b)].astype(F32)
                                for half in range(2)], axis=0).reshape(4, 8, D)

    def mean_rows(i, b):
        stats[i, b] = _row_sum(load_rows(i, b)) * (1.0 / D)
        return _row_token(stats[i, b])

    def spread_rows(i, b):
        stats[i, b] = stats[i, b], _inv_std(load_rows(i, b) - stats[i, b])
        return _row_token(stats[i, b][1])

    def normalize_rows(i, b):
        mean, inv = stats.pop((i, b))
        x = load_rows(i, b)
        parts = []
        for l in range(HALF // 128):
            lo, hi = (((x[:, :, c0:c0 + 128] - mean) * inv * mod_a[at(1), :, c0:c0 + 128][None]
                       + mod_a[at(0), :, c0:c0 + 128][None]).reshape(32, 128)
                      for c0 in (l * 128, HALF + l * 128))
            parts.append(_right_operands(lo[:16], lo[16:], hi[:16], hi[16:]))
        h_parts[i, b] = [jnp.concatenate([p[n] for p in parts], axis=1) for n in range(NOPS)]

    def spread_and_normalize(i, b):
        token = spread_rows(i, b)
        normalize_rows(i, b)
        return token

    def h_operand(i, n):
        if (i, n) not in h_ops:
            h_ops[i, n] = jnp.concatenate([h_parts[i, b][n] for b in range(8)], axis=0).astype(BF16)
        return h_ops[i, n]

    def project(w_s, sg, i, tasks):
        blocks = block_product(lambda n: w_s[at(sg * NOPS + n)], lambda n: h_operand(i, n), _NT, tasks)
        return [[blocks[j // 2 * 2 + half][(j % 2) * 64:(j % 2 + 1) * 64] for half in range(2)]
                for j in range(4)]

    def key_features(p, pair, i, out):
        (phi0, token0), (phi1, token1) = _feature_map(p[0]), _feature_map(p[1])
        z_acc[pair] = phi0 + phi1 if i == 0 else z_acc[pair] + phi0 + phi1
        out.append(jnp.concatenate([phi0, phi1], axis=1).astype(BF16))
        return token0 | token1

    def accumulate_kv(v, phi, sg, i):
        for j in range(4):
            kv = _dot(jnp.concatenate(v[j], axis=1).astype(BF16), phi[j], _NT)
            kv_acc[4 * sg + j] = kv if i == 0 else kv_acc[4 * sg + j] + kv

    cp_x[0].wait()
    for b in range(8):
        mean_rows(0, b)
    for b in range(8):
        spread_rows(0, b)
    cp_phi.wait()
    phi_bd = phi_blocks()
    for k, cp in enumerate(cp_mod_a):
        cp.wait()
        modulation(k * MOD_CHUNK)
    for b in range(8):
        normalize_rows(0, b)

    task = functools.partial
    pending = None
    for u in range(UNITS):
        i, sg = divmod(u, SG)
        if i == 0:
            cp_wk[sg].wait()
            if sg == 2:
                cp_x[1].wait()
            if sg > 0:
                cp_wv[sg].wait()
            for l in range(HALF // 128):
                fold_phi(D, wk_s, sg, l)
        if u == SG:
            cp_x[2].wait()
        if u == 2 * SG:
            cp_x[3].wait()
        if u == FOLD_Q_UNIT:
            cp_wq.wait()
            cp_wr.wait()
        if u == MOD_UNIT:
            cp_mod_b.wait()
            cp_wo.wait()
        if FOLD_Q_UNIT <= u < FOLD_Q_UNIT + 8:
            k = 2 * (u - FOLD_Q_UNIT)
            fold_phi(0, wq_s, *divmod(k, 4))
            fold_phi(0, wq_s, *divmod(k + 1, 4))
        if MOD_UNIT <= u < MOD_UNIT + 4:
            for k in range(4):
                modulation(2 * D + (4 * (u - MOD_UNIT) + k) * MOD_CHUNK)

        if i == 0:
            blocks = range(4 * (sg - 2), 4 * (sg - 1)) if sg >= 2 else ()
        else:
            blocks = (2 * sg, 2 * sg + 1) if i + 1 < TILES else ()
        first, last = [], []
        for k, b in enumerate(blocks):
            (first if k < 2 else last).extend(
                [(LN_SLOTS[k % 2 * 2], task(mean_rows, i + 1, b)),
                 (LN_SLOTS[k % 2 * 2 + 1], task(spread_and_normalize, i + 1, b))])
        pk = project(wk_s, sg, i, first)
        if i == 0:
            if sg == 0:
                cp_wv[0].wait()
            transpose_wv(sg)
        if pending is not None:
            accumulate_kv(*pending)
        phi = []
        last += [(KEY_SLOTS[j], task(key_features, pk[j], 4 * sg + j, i, phi)) for j in range(4)]
        if i == TILES - 1:
            last += [(2 + k, task(split_wo, sg, k, _bits(pk[k][0][:8]))) for k in range(4)]
        pending = (project(wv_s, sg, i, last), phi, sg, i)
    accumulate_kv(*pending)

    same_head = _iota((64, 128), 0) // DH == _iota((64, 128), 1) % 2
    head_rows = _iota((16, 128), 0) // 8 == _iota((16, 128), 1) % 2
    kvT = []
    for pair in range(PAIRS):
        z = jnp.sum(z_acc[pair].T, axis=0, keepdims=True)
        kvT.append(jnp.concatenate(
            [jnp.where(same_head, kv_acc[pair], 0.0), jnp.where(head_rows, z, 0.0)],
            axis=0).astype(BF16))

    wr = wr_v[...].astype(F32)
    wr = jnp.concatenate([jnp.broadcast_to(wr[l:l + 1, :], (8, 128)) for l in range(D // 128)], axis=1)
    shift, scale, gate_b = mod_b[1], mod_b[2], mod_b[3]
    score_bias = _row_sum(shift * wr)
    mod_b[4] = scale * wr
    mod_b[5] = scale * gate_b
    mod_b[6] = shift * gate_b

    def query_features(p, out):
        (phi0, token0), (phi1, token1) = _feature_map(p[0]), _feature_map(p[1])
        out.append(jnp.concatenate([phi0, phi1], axis=1).astype(BF16))
        return token0 | token1

    def attend(feats, sg):
        return [_dot(kvT[4 * sg + j], feats[j], _NN) for j in range(4)]

    o_parts, o_ops = {}, {}

    def o_operand(i, n):
        if (i, n) not in o_ops:
            o_ops[i, n] = jnp.concatenate([o_parts[i, sg][n] for sg in range(SG)], axis=1).astype(BF16)
        return o_ops[i, n]

    def store_attention(nums, sg, i):
        blocks = []
        for num in nums:
            num = num.reshape(10, 8, T)
            inv = _recip(num[8:] + 1e-6)
            o = jnp.concatenate([num[:4] * inv[0:1], num[4:8] * inv[1:2]], axis=0)
            blocks.append(o.reshape(64, T))
        first = jnp.concatenate(blocks[:2], axis=0).T
        second = jnp.concatenate(blocks[2:], axis=0).T
        quads = first[:128], second[:128], first[128:], second[128:]
        o_parts[i, sg] = _left_operands(*quads)
        return _join([_bits(q[120:]) for q in quads])

    def project_out(i, cp, tasks):
        return block_product(lambda n: o_operand(i, n), lambda n: wo_s[at(cp * NOPS + n)], _NN, tasks)

    def add_residual(blocks, i, cp):
        for k, attn in enumerate(blocks):
            cs = pl.ds(cp * 256 + (k % 2) * 128, 128)
            x = x_v[pl.ds(at(i * 16 + (k // 2) * 8), 8), :, cs].astype(F32).reshape(16, 8, 128)
            x1 = x + mod_b[at(0), :, cs][None] * attn.reshape(16, 8, 128)
            x1_v[i][(k // 2) * 8:(k // 2 + 1) * 8, :, cs] = x1.reshape(8, 16, 128)

    top = [jnp.full((8, 128), -jnp.inf, F32), jnp.zeros((8, 128), I32)] * 2

    def load_attended(r0, n):
        return x1_v[r0 // T][pl.ds(at(r0 % T // 16), n // 16)].reshape(n // 8, 8, D)

    def mean_attended(r0, n):
        stats[r0] = _row_sum(load_attended(r0, n)) * (1.0 / D)
        return _row_token(stats[r0])

    def finish_rows(r0, n):
        mean = stats.pop(r0)
        centered = load_attended(r0, n) - mean
        routed = _row_sum(centered * mod_b[at(4)][None])
        inv = _inv_std(centered)
        x1 = load_attended(r0, n)
        out = x1 + ((x1 - mean) * inv * mod_b[at(5)][None] + mod_b[at(6)][None])
        out_v[pl.ds(r0 // 16, n // 16)] = out.reshape(n // 16, 16, D).astype(BF16)
        score = _round_bf16(routed * inv + score_bias)
        best, best_i, second, second_i = top
        for b in range(n // 8):
            s, t = jnp.broadcast_to(score[b], (8, 128)), _iota((8, 128), 0) + (r0 + 8 * b)
            above_best, above_second = s > best, s > second
            second = jnp.where(above_best, best, jnp.where(above_second, s, second))
            second_i = jnp.where(above_best, best_i, jnp.where(above_second, t, second_i))
            best = jnp.where(above_best, s, best)
            best_i = jnp.where(above_best, t, best_i)
        top[:] = best, best_i, second, second_i
        return _bits(second_i)

    def run(tasks):
        for _, fn in sorted(tasks, key=lambda item: item[0]):
            fn()

    feats = attn = None
    for u in range(UNITS + SG):
        first, last = [], []
        if feats is not None:
            tile, sg = divmod(u - 1, SG)
            first.append((STORE_SLOT, task(store_attention, attend(feats, sg), sg, tile)))
        if attn is not None:
            add_residual(attn, *divmod(u - SG - 1, SG))
        if u >= 2 * SG:
            for k, slots in enumerate(FINISH_SLOTS):
                r0 = (u - 2 * SG) * 64 + 16 * k
                for slot, fn in zip(slots, (mean_attended, finish_rows)):
                    if u >= UNITS:
                        last.append((slot * 6 // 8, task(fn, r0, 16)))
                    else:
                        (first if slot < 7 else last).append((slot % 7, task(fn, r0, 16)))
        feats = attn = None
        if u < UNITS:
            tile, sg = divmod(u, SG)
            pq = project(wq_s, sg, tile, first)
            feats = []
            last += [(QUERY_SLOTS[j], task(query_features, pq[j], feats)) for j in range(4)]
        else:
            run(first)
        if u >= SG:
            attn = project_out(*divmod(u - SG, SG), last)
        else:
            run(last)
        if u >= 2 * SG and u % SG == SG - 1:
            cp_out[u // SG - 2].start()
    add_residual(attn, TILES - 1, SG - 1)
    for fn in (mean_attended, finish_rows):
        for r0 in range(S - T, S, LAST_ROWS):
            fn(r0, LAST_ROWS)
    cp_out[TILES - 1].start()
    best, best_i, second, second_i = top

    scores = jnp.concatenate([best, second], axis=0)
    tokens = jnp.concatenate([best_i, second_i], axis=0)

    def take_top(scores):
        top = jnp.max(scores, axis=0, keepdims=True)
        tok = jnp.min(jnp.where(scores == top, tokens, S - 1).astype(F32), axis=0, keepdims=True)
        return top, tok.astype(I32)

    score0, tok0 = take_top(scores)
    score1, tok1 = take_top(jnp.where(tokens == tok0, -jnp.inf, scores))
    idx = [jnp.clip(tok0[0, 0], 0, S - 1), jnp.clip(tok1[0, 0], 0, S - 1)]
    base = [t // 16 for t in idx]

    for k in range(2):
        for i in range(TILES):
            @pl.when(base[k] // 16 == i)
            def _():
                picked_v[k] = x1_v[i][base[k] % 16]

    row16 = _iota((16, D), 0)
    x1_blk, h2_blk = [], []
    h_sel = jnp.zeros((16, D), F32)
    for k in range(2):
        x1 = picked_v[k]
        centered = x1.reshape(2, 8, D)
        centered = centered - _row_sum(centered) * (1.0 / D)
        h2 = (centered * _inv_std(centered) * scale[None] + shift[None]).reshape(16, D)
        picked = jnp.sum(jnp.where(row16 == idx[k] % 16, h2, 0.0), axis=0, keepdims=True)
        h_sel = jnp.where(row16 == k, picked, h_sel)
        x1_blk.append(x1)
        h2_blk.append(h2)
    h_sel = h_sel.astype(BF16)

    for cp in cp_ffn:
        cp.wait()
    y = jnp.zeros((16, D), F32)
    for f in range(F // F_CHUNK):
        sl = slice(f * F_CHUNK, (f + 1) * F_CHUNK)
        gate = _dot(h_sel, wg_v[:, sl], _NN)
        up = _dot(h_sel, wu_v[:, sl], _NN)
        act = (gate * jax.nn.sigmoid(gate) * up).astype(BF16)
        y = y + _dot(act, wd_v[sl, :], _NN)
    y_sel = [y[0:1] * jax.nn.sigmoid(score0[:, :1]), y[1:2] * jax.nn.sigmoid(score1[:, :1])]

    for cp in cp_out:
        cp.wait()

    gb = jnp.concatenate([gate_b, gate_b], axis=0)
    for k in range(2):
        upd = jnp.zeros((16, D), F32)
        for m in range(2):
            upd = jnp.where(row16 == idx[m] - 16 * base[k], y_sel[m], upd)
        out_v[base[k]] = (x1_blk[k] + gb * (h2_blk[k] + upd)).astype(BF16)

    fix = [copy(out_v.at[base[k]], out_hbm.at[base[k]]) for k in range(2)]
    fix[0].start()

    @pl.when(base[0] != base[1])
    def _():
        fix[1].start()
        fix[1].wait()

    fix[0].wait()


@jax.jit
def pallas_adaLN_cond__linear_kernel_hedgehog__moe_arch_mod__prompt_kernel(
    A_x: jax.Array,
    A_wqkv: jax.Array,
    A_w_phi: jax.Array,
    A_wo: jax.Array,
    B_x: jax.Array,
    B_w_r: jax.Array,
    B_w_gate: jax.Array,
    B_w_up: jax.Array,
    B_w_down: jax.Array,
    c: jax.Array,
    w_mod: jax.Array,
):
    del B_x
    weight_operands = pltpu.VMEM((SG * NOPS, 64, HALF), U32)
    out = pl.pallas_call(
        _kernel,
        out_shape=jax.ShapeDtypeStruct((S // 16, 16, D), BF16),
        in_specs=[pl.BlockSpec(memory_space=pl.ANY)] * 10,
        out_specs=pl.BlockSpec(memory_space=pl.ANY),
        scratch_shapes=[
            pltpu.VMEM((S // 16, 16, D), BF16),
            pltpu.VMEM((D, 3 * D), BF16),
            pltpu.VMEM((H * DH, DH), BF16),
            pltpu.VMEM((SG + 1, 256, D), BF16),
            pltpu.VMEM((D // 128, 128), BF16),
            pltpu.VMEM((D, F), BF16),
            pltpu.VMEM((D, F), BF16),
            pltpu.VMEM((F, D), BF16),
            pltpu.VMEM((1, D), BF16),
            pltpu.VMEM((D, 6 * D), BF16),
            weight_operands,
            weight_operands,
            weight_operands,
            pltpu.VMEM((SG * NOPS, HALF // 2, 128), U32),
            pltpu.VMEM((2, 16, D), F32),
            pltpu.VMEM((S // 16, 16, D), BF16),
            pltpu.VMEM((2, 8, D), F32),
            pltpu.VMEM((7, 8, D), F32),
            pltpu.VMEM((PAIRS, 64, 128), F32),
            pltpu.VMEM((PAIRS, 128, 128), F32),
            pltpu.SemaphoreType.DMA((48,)),
            *[pltpu.VMEM((T // 16, 16, D), F32)] * TILES,
        ],
        compiler_params=pltpu.CompilerParams(vmem_limit_bytes=120 * 1024 * 1024),
        name="hedgehog_moe",
    )(
        A_x.reshape(S // 16, 16, D), A_wqkv, A_w_phi.reshape(H * DH, DH),
        A_wo.reshape(SG, 256, D), B_w_r.reshape(D // 128, 128), B_w_gate, B_w_up, B_w_down, c, w_mod,
    )
    return out.reshape(1, S, D)
```

```python
import functools
import itertools
import math

import jax
import jax.numpy as jnp
from jax import lax
import jax.experimental.pallas as pl
import jax.experimental.pallas.tpu as pltpu

S, D, H, DH, F = 2048, 1024, 32, 32, 3584
PAIRS = H // 2
T = 256
TILES = S // T
SG = 4
UNITS = TILES * SG
HALF = D // 2
F_CHUNK = 512
MOD_CHUNK = 256
LOG2E = math.log2(math.e)
NOPS = 7

KEY_SLOTS = (2, 3, 5, 6)
QUERY_SLOTS = (2, 3, 4, 5)
LN_SLOTS = (13, 3)
LN_EARLY_SLOTS = (0, 4, 8, 12)
LN_SLACK = 3
STORE_SLOT = 6
VALUE_SLOT = 2
FINISH_SLOTS = ((1, 3), (2, 4), (5, 7), (6, 8))
LATE_UNIT = UNITS - 12 if UNITS > 20 else UNITS - 8
EARLY_OUT = max(TILES - 3, 1)
LAST_ROWS = 64
OUT_CHUNK = 2
LEAD1 = 5
PACE = 12
NORM_BACK = 2
LEAD2 = 5
HOLD = 'orqm'

F32 = jnp.float32
BF16 = jnp.bfloat16
U32 = jnp.uint32
I32 = jnp.int32

_NN = (((1,), (0,)), ((), ()))
_NT = (((1,), (1,)), ((), ()))


def _dot(a, b, dims):
    return lax.dot_general(a, b, dims, preferred_element_type=F32)


def _round_bf16(x):
    return x.astype(BF16).astype(F32)


def _bits(x):
    return pltpu.bitcast(x, U32)


def _iota(shape, axis):
    return lax.broadcasted_iota(I32, shape, axis)


def _recip(x):
    return pl.reciprocal(x, full_range=False)


def _join(tokens):
    return functools.reduce(jnp.bitwise_or, tokens)


def _left_operands(a11, a12, a21, a22):
    return a11 + a22, a21 + a22, a11, a22, a11 + a12, a21 - a11, a12 - a22


def _right_operands(b11, b12, b21, b22):
    return b11 + b22, b11, b12 - b22, b21 - b11, b22, b11 + b12, b21 + b22


def _row_sum(x):
    return jnp.sum(x, axis=-1, keepdims=True)


def _inv_std(centered):
    return lax.rsqrt(_row_sum(centered * centered) * (1.0 / D) + 1e-5)


def _row_token(x):
    return _join([_bits(jnp.broadcast_to(x[i], (8, 128))) for i in range(x.shape[0])])


def _transposed_words(x):
    return _bits(x.astype(BF16).T)


def _head_allreduce(x, op):
    r = functools.reduce(op, [x[i:i + 8] for i in range(0, 64, 8)])
    r = op(r, pltpu.roll(r, 4, 0))
    return op(r, pltpu.roll(r, 2, 0))


def _feature_map(p):
    p3 = p.reshape(8, 8, T)
    e_pos = jnp.exp2(p3 - _head_allreduce(p, jnp.maximum)[None])
    e_neg = jnp.exp2(_head_allreduce(p, jnp.minimum)[None] - p3)
    inv_pos, inv_neg = (_recip(_head_allreduce(e.reshape(64, T), jnp.add)) for e in (e_pos, e_neg))
    phi = jnp.concatenate([e_pos * inv_pos[None], e_neg * inv_neg[None]], axis=0)
    token = _bits(inv_pos) | _bits(inv_neg)
    return phi.reshape(128, T).astype(BF16), token[:, :128] | token[:, 128:]


def _kernel(x_hbm, wqkv_hbm, wphi_hbm, wo_hbm, wr_hbm, wg_hbm, wu_hbm, wd_hbm, c_hbm, wmod_hbm,
            out_hbm,
            x_v, wqkv_v, wphi_v, wo_v, wr_v, wg_v, wu_v, wd_v, c_v, wmod_v,
            wq_s, wk_s, wv_s, wo_s, out_v, mod_a, mod_b, phi_s, v_s, kv_s, stat_v,
            sems, *rest):
    x1_v, kv_acc, h_s = rest[:2], rest[2:6], rest[6:]
    sem_ids = itertools.count()

    def copy(src, dst):
        return pltpu.make_async_copy(src, dst, sems.at[next(sem_ids)])

    def copy_slabs(src, dst, first, count):
        sem = sems.at[next(sem_ids)]
        return [pltpu.make_async_copy(src.at[:, pl.ds(k * 128, 128)], dst.at[k], sem)
                for k in range(first, first + count)]

    def wait_all(copies):
        for cp in copies:
            cp.wait()

    def copy_blocks(src, dst, start, size):
        return copy(src.at[pl.ds(start, size)], dst.at[pl.ds(start, size)])

    cp_c, cp_phi, cp_wr = copy(c_hbm, c_v), copy(wphi_hbm, wphi_v), copy(wr_hbm, wr_v)
    cp_x = [copy_blocks(x_hbm, x_v, 16 * i, 16) for i in range(2)]
    cp_x.append(copy_blocks(x_hbm, x_v, 32, S // 16 - 32))
    cp_mod_a = [copy_slabs(wmod_hbm, wmod_v, k, 2) for k in range(0, 16, 2)]
    cp_wk = [copy_slabs(wqkv_hbm, wqkv_v, 8 + 2 * sg, 2) for sg in range(SG)]
    cp_wv = [copy_slabs(wqkv_hbm, wqkv_v, 16 + 2 * sg, 2) for sg in range(SG)]
    cp_wq = copy_slabs(wqkv_hbm, wqkv_v, 0, 8)
    cp_late = copy_slabs(wmod_hbm, wmod_v, 16, 32) + [cp_wr, copy_blocks(wo_hbm, wo_v, 0, SG)]
    cp_ffn = [copy(wg_hbm, wg_v), copy(wu_hbm, wu_v), copy(wd_hbm, wd_v)]
    cp_out = [copy_blocks(out_v, out_hbm, 0, 16 * EARLY_OUT),
              copy_blocks(out_v, out_hbm, 16 * EARLY_OUT, 16 * (TILES - EARLY_OUT))]
    for cp in (cp_c, cp_x[0], cp_phi, *itertools.chain(*cp_mod_a), *cp_wk[0], *cp_wv[0], *cp_wk[1],
               *cp_wv[1], cp_x[1], *cp_wk[2], *cp_wv[2], *cp_wk[3], *cp_wv[3], cp_x[2], *cp_wq, *cp_late, *cp_ffn):
        cp.start()

    cp_c.wait()
    c = c_v[...].astype(F32)
    silu_c = jnp.broadcast_to(c * jax.nn.sigmoid(c), (16, D)).astype(BF16)
    never = jnp.broadcast_to(c[:, :128] * c[:, :128], (8, 128)) < 0.0
    zero = jnp.max(never.astype(F32)).astype(I32)
    stamps = itertools.count(1)

    def at(i):
        return i + zero * next(stamps)

    def after(words, token):
        head = jnp.concatenate([jnp.where(never, token, words[:8, l:l + 128])
                                for l in range(0, words.shape[1], 128)], axis=1)
        return jnp.concatenate([head, words[8:]], axis=0)

    def hold(ref, token):
        token = pltpu.bitcast(token, ref.dtype)
        ref[ref.shape[0] - 1, :token.shape[0], :128] = token

    def once(value, token):
        return jnp.where(never[:, :1], token, value)

    history, due = [], {}

    def tick(back, step):
        back, step = back - step // 16, step % 16
        return history[-back][8 * step:8 * step + 8, :128]

    def block_product(left, right, dims, tasks):
        def m(n, slot):
            for at_slot, fn, *slack in tasks:
                if at_slot == slot:
                    due.setdefault(len(history) + sum(slack), []).append(fn())
            tokens = [t for t in due.pop(len(history), []) if t is not None]
            operands = [left(n), right(n)]
            for k, op in enumerate(operands):
                if op.dtype == U32:
                    operands[k] = pltpu.bitcast(after(op, _join(tokens)) if tokens else op, BF16)
            result = _dot(*operands, dims)
            history.append(result)
            return result

        m2, m4 = m(1, 0), m(3, 1)
        c21 = m2 + m4
        m3 = m(2, 2)
        c22 = m3 - m2
        m5 = m(4, 3)
        c12 = m3 + m5
        c11 = m4 - m5
        m1 = m(0, 4)
        c11, c22 = c11 + m1, c22 + m1
        c11 = c11 + m(6, 5)
        c22 = c22 + m(5, 6)
        return c11, c12, c21, c22

    def modulation(col0):
        i, c0 = divmod(col0, D)
        w = jnp.concatenate([wmod_v[at(col0 // 128 + k)] for k in range(2)], axis=1)
        m = _round_bf16(_dot(silu_c, w, _NN)[:8])
        dst, row = (mod_a, i) if i < 2 else (mod_b, i - 2)
        dst[row, :, c0:c0 + MOD_CHUNK] = _round_bf16(1.0 + m) if i % 3 == 1 else m

    def phi_blocks():
        select = (_iota((128, DH), 0) % 64 // 2 == _iota((128, DH), 1)).astype(BF16)
        row = _iota((128, 128), 0)
        same_head = row // 64 * 2 + row % 2 == _iota((128, 128), 1) // DH
        return [jnp.where(same_head, _dot(select, wphi_v[g * 128:(g + 1) * 128, :], _NT), 0.0)
                .astype(BF16) for g in range(D // 128)]

    def fold_phi(col0, dst, sg, l):
        quads = []
        for g in (2 * sg, 2 * sg + 1):
            w = jnp.concatenate([wqkv_v[at(col0 // 128 + g), r:r + 128, :]
                                 for r in (l * 128, HALF + l * 128)], axis=0)
            folded = _dot(phi_bd[g], w, _NT) * LOG2E
            quads += [folded[:, :128], folded[:, 128:]]
        for n, op in enumerate(_left_operands(*quads)):
            dst[sg * NOPS + n, :, l * 128:(l + 1) * 128] = _bits(op.astype(BF16))

    def transpose_wv(sg):
        first, second = (wqkv_v[at(16 + 2 * sg + k)].astype(F32) for k in range(2))
        ops = _left_operands(first[:HALF], first[HALF:], second[:HALF], second[HALF:])
        for n, op in enumerate(ops):
            wv_s[sg * NOPS + n] = _transposed_words(op)

    def split_wo(cp, sg, token):
        hold(wo_v, token)
        w = wo_v[at(sg), :, cp * 256:(cp + 1) * 256].astype(F32)
        ops = _right_operands(w[:128, :128], w[:128, 128:], w[128:, :128], w[128:, 128:])
        for n, op in enumerate(ops):
            wo_s[cp * NOPS + n, :, sg * 128:(sg + 1) * 128] = _transposed_words(op)

    stats = {}

    def load_rows(i, b):
        return jnp.concatenate([x_v[at(i * 16 + half * 8 + b)].astype(F32)
                                for half in range(2)], axis=0).reshape(4, 8, D)

    def paced(stat, back, step):
        return once(stat, tick(back, step)[None, :, :1]) if back else stat

    def mean_rows(i, b, back=0):
        if back:
            hold(x_v, tick(back, 0))
        stats[i, b] = _row_sum(load_rows(i, b)) * (1.0 / D)

    def spread_rows(i, b):
        stats[i, b] = stats[i, b], _inv_std(load_rows(i, b) - stats[i, b])

    def normalize_rows(i, b, back=0):
        mean, inv = stats.pop((i, b))
        mean = once(mean, inv)
        x = load_rows(i, b)
        for l in range(HALF // 256):
            m = paced(mean, back, PACE * l)
            lo, hi = (((x[:, :, c0:c0 + 256] - m) * inv * mod_a[at(1), :, c0:c0 + 256][None]
                       + mod_a[at(0), :, c0:c0 + 256][None]).reshape(32, 256)
                      for c0 in (l * 256, HALF + l * 256))
            for n, op in enumerate(_right_operands(lo[:16], lo[16:], hi[:16], hi[16:])):
                h_s[i][n, 16 * b:16 * (b + 1), l * 256:(l + 1) * 256] = op.astype(BF16)

    def layer_norm_rows(i, b):
        mean_rows(i, b, LEAD1)
        spread_rows(i, b)
        normalize_rows(i, b, NORM_BACK)
        return _bits(h_s[i][at(0), 16 * b:16 * (b + 1), :128])

    def project(w_s, sg, i, tasks):
        blocks = block_product(lambda n: w_s[at(sg * NOPS + n)], lambda n: h_s[i][at(n)], _NT, tasks)
        return [[blocks[j // 2 * 2 + half][(j % 2) * 64:(j % 2 + 1) * 64] for half in range(2)]
                for j in range(4)]

    def key_features(p, out):
        phi, token = _feature_map(jnp.concatenate(p, axis=1))
        out.append(phi)
        return token

    def store_values(v):
        for j in range(4):
            v_s[j, :64, :] = jnp.concatenate(v[j], axis=1).astype(BF16)
        return _bits(v_s[at(0), :16, :128])

    def accumulate_kv(sg, i, phi):
        for j in range(4):
            kv = _dot(v_s[at(j)], phi[j], _NT)
            kv = kv if i == 0 else kv_acc[j][at(sg)] + kv
            if i + 1 < TILES:
                kv_acc[j][sg] = kv
            else:
                row = _iota((80, 128), 0)
                head = jnp.where(row < 64, row // DH, row // 8 % 2)
                kv_s[4 * sg + j] = jnp.where(head == _iota((80, 128), 1) % 2, kv, 0.0).astype(BF16)

    v_s[:, 64:, :] = jnp.ones((4, 16, T), BF16)

    cp_x[0].wait()
    for b in range(8):
        mean_rows(0, b)
    for b in range(8):
        spread_rows(0, b)
    cp_phi.wait()
    phi_bd = phi_blocks()
    for k, cp in enumerate(cp_mod_a):
        wait_all(cp)
        modulation(k * MOD_CHUNK)
    for b in range(8):
        normalize_rows(0, b)

    task = functools.partial
    pending = None
    for u in range(UNITS):
        i, sg = divmod(u, SG)
        if i == 0:
            wait_all(cp_wk[sg])
            if sg == 2:
                cp_x[1].wait()
            if sg > 0:
                wait_all(cp_wv[sg])
            for l in range(HALF // 128):
                fold_phi(D, wk_s, sg, l)
        if u == SG + 2:
            cp_x[2].wait()
        if u == LATE_UNIT:
            wait_all(cp_late)
            wait_all(cp_wq)
        if LATE_UNIT <= u < LATE_UNIT + 8:
            k = 2 * (u - LATE_UNIT)
            if 'q' in HOLD:
                hold(wqkv_v, _bits(pk[0][1][:8]))
            fold_phi(0, wq_s, *divmod(k, 4))
            fold_phi(0, wq_s, *divmod(k + 1, 4))
            for k in range(2):
                modulation(2 * D + (2 * (u - LATE_UNIT) + k) * MOD_CHUNK)

        if i < 2:
            blocks = range(4 * (sg - 2), 4 * (sg - 1)) if sg >= 2 else ()
        else:
            blocks = (2 * sg, 2 * sg + 1) if i + 1 < TILES else ()
        first, last = [], []
        for k, b in enumerate(blocks):
            slot = (LN_SLOTS if i >= 2 else LN_EARLY_SLOTS)[k]
            (first if slot < 7 else last).append((slot % 7, task(layer_norm_rows, i + 1, b), LN_SLACK))
        if pending is not None:
            first.append((VALUE_SLOT, task(store_values, pending[0])))
        pk = project(wk_s, sg, i, first)
        if i == 0:
            if sg == 0:
                wait_all(cp_wv[0])
            transpose_wv(sg)
        if pending is not None:
            accumulate_kv(*pending[1:])
        phi = []
        last += [(KEY_SLOTS[j], task(key_features, pk[j], phi)) for j in range(4)]
        if i == TILES - 1:
            last += [(2 + k, task(split_wo, sg, k, _bits(pk[k][0][:8]))) for k in range(4)]
        pending = (project(wv_s, sg, i, last), sg, i, phi)
    store_values(pending[0])
    accumulate_kv(*pending[1:])

    wr = wr_v[...].astype(F32)
    wr = jnp.concatenate([jnp.broadcast_to(wr[l:l + 1, :], (8, 128)) for l in range(D // 128)], axis=1)
    shift, scale, gate_b = mod_b[1], mod_b[2], mod_b[3]
    score_bias = _row_sum(shift * wr)
    mod_b[4] = scale * wr
    mod_b[5] = scale * gate_b
    mod_b[6] = shift * gate_b

    def query_features(p, out):
        phi, token = _feature_map(jnp.concatenate(p, axis=1))
        out.append(phi)
        return token

    def attend(feats, sg, out):
        out.extend(_dot(kv_s[at(4 * sg + j)], feats[j], _NN) for j in range(4))

    o_parts, o_ops = {}, {}

    def o_operand(i, n):
        if (i, n) not in o_ops:
            o_ops[i, n] = jnp.concatenate([o_parts[i, sg][n] for sg in range(SG)], axis=1).astype(BF16)
        return o_ops[i, n]

    def store_attention(nums, sg, i):
        blocks = []
        for num in nums:
            num = num.reshape(10, 8, T)
            inv = _recip(num[8:] + 1e-6)
            o = jnp.concatenate([num[:4] * inv[0:1], num[4:8] * inv[1:2]], axis=0)
            blocks.append(o.reshape(64, T))
        first = jnp.concatenate(blocks[:2], axis=0).T
        second = jnp.concatenate(blocks[2:], axis=0).T
        quads = first[:128], second[:128], first[128:], second[128:]
        o_parts[i, sg] = _left_operands(*quads)
        return _join([_bits(q[120:]) for q in quads])

    def project_out(i, cp, tasks):
        return block_product(lambda n: o_operand(i, n), lambda n: wo_s[at(cp * NOPS + n)], _NT, tasks)

    def add_residual(blocks, i, cp):
        for k in (2, 1, 0, 3):
            attn = blocks[k]
            if 'r' in HOLD:
                hold(x_v, _bits(attn[:8]))
            cs = pl.ds(cp * 256 + (k % 2) * 128, 128)
            x = x_v[pl.ds(at(i * 16 + (k // 2) * 8), 8), :, cs].astype(F32).reshape(16, 8, 128)
            x1 = x + mod_b[at(0), :, cs][None] * attn.reshape(16, 8, 128)
            x1_v[i % 2][pl.ds(i // 2 * 16 + (k // 2) * 8, 8), :, cs] = x1.reshape(8, 16, 128)

    top = [jnp.full((8, 128), -jnp.inf, F32), jnp.zeros((8, 128), I32)] * 2

    def load_attended(r0, n):
        i = r0 // T
        return x1_v[i % 2][pl.ds(at(i // 2 * 16 + r0 % T // 16), n // 16)].reshape(n // 8, 8, D)

    def mean_attended(r0, n):
        if n == 16 and LEAD2:
            hold(x1_v[r0 // T % 2], tick(LEAD2, 0))
        stats[r0] = _row_sum(load_attended(r0, n)) * (1.0 / D)
        return _row_token(stats[r0])

    def score_rows(r0, n):
        mean = stats.pop(r0)
        centered = load_attended(r0, n) - mean
        routed = _row_sum(centered * mod_b[at(4)][None])
        inv = _inv_std(centered)
        for k, stat in enumerate((mean, inv)):
            stat_v[k, pl.ds(r0 // 8, n // 8)] = jnp.broadcast_to(stat, (n // 8, 8, 128))
        stats[r0] = mean, inv
        score = _round_bf16(routed * inv + score_bias)
        best, best_i, second, second_i = top
        for b in range(n // 8):
            s, t = jnp.broadcast_to(score[b], (8, 128)), _iota((8, 128), 0) + (r0 + 8 * b)
            above_best, above_second = s > best, s > second
            second = jnp.where(above_best, best, jnp.where(above_second, s, second))
            second_i = jnp.where(above_best, best_i, jnp.where(above_second, t, second_i))
            best = jnp.where(above_best, s, best)
            best_i = jnp.where(above_best, t, best_i)
        top[:] = best, best_i, second, second_i

    def output_rows(r0, n, token=None):
        mean, inv = stats.pop(r0)
        if token is not None:
            inv = once(inv, token[None])
        x1 = load_attended(r0, n)
        out = x1 + ((x1 - once(mean, inv)) * inv * mod_b[at(5)][None] + mod_b[at(6)][None])
        out_v[pl.ds(r0 // 16, n // 16)] = out.reshape(n // 16, 16, D).astype(BF16)

    def finish_rows(r0, n):
        score_rows(r0, n)
        output_rows(r0, n)
        return _bits(top[3]) | _bits(out_v[at(0), :, :128])

    def run(tasks):
        for _, fn, *_ in sorted(tasks, key=lambda item: item[0]):
            fn()

    feats = attn = None
    for u in range(UNITS + SG):
        first, last = [], []
        if feats is not None:
            tile, sg = divmod(u - 1, SG)
            nums = []
            first.append((3 if u <= SG else 0, task(attend, feats, sg, nums)))
            first.append((STORE_SLOT, task(store_attention, nums, sg, tile)))
        if attn is not None:
            add_residual(attn, *divmod(u - SG - 1, SG))
        if u >= 2 * SG:
            for k, slots in enumerate(FINISH_SLOTS):
                r0 = (u - 2 * SG) * 64 + 16 * k
                for slot, fn in zip(slots, (mean_attended, finish_rows)):
                    if u >= UNITS:
                        last.append((slot * 6 // 8, task(fn, r0, 16)))
                    else:
                        (first if slot < 7 else last).append((slot % 7, task(fn, r0, 16)))
        feats = attn = None
        if u < UNITS:
            tile, sg = divmod(u, SG)
            pq = project(wq_s, sg, tile, first)
            feats = []
            last += [(QUERY_SLOTS[j], task(query_features, pq[j], feats)) for j in range(4)]
        else:
            run(first)
        if u >= SG:
            attn = project_out(*divmod(u - SG, SG), last)
        else:
            run(last)
        if u == (EARLY_OUT + 2) * SG - 1:
            cp_out[0].start()
            wait_all(cp_ffn)
    add_residual(attn, TILES - 1, SG - 1)
    for fn in (mean_attended, score_rows):
        for r0 in range(S - T, S, LAST_ROWS):
            fn(r0, LAST_ROWS)
    best, best_i, second, second_i = top

    scores = jnp.concatenate([best, second], axis=0)
    tokens = jnp.concatenate([best_i, second_i], axis=0)

    def take_top(scores):
        top = jnp.max(scores, axis=0, keepdims=True)
        tok = jnp.min(jnp.where(scores == top, tokens, S - 1).astype(F32), axis=0, keepdims=True)
        return top, tok.astype(I32)

    score0, tok0 = take_top(scores)
    score1, tok1 = take_top(jnp.where(tokens == tok0, -jnp.inf, scores))
    routed = [jnp.clip(tok[0, 0], 0, S - 1) for tok in (tok0, tok1)]

    row16 = _iota((16, D), 0)
    x1_sel = h2_sel = weight = jnp.zeros((16, D), F32)
    for k, (t, score) in enumerate(zip(routed, (score0, score1))):
        blk, row = t // (2 * T) * 16 + t % T // 16, pl.ds(t % 16, 1)
        x1 = jnp.where(t // T % 2 == 0, x1_v[0][blk, row, :], x1_v[1][blk, row, :])
        mean, inv = (jnp.tile(stat_v[m, t // 8, pl.ds(t % 8, 1), :], (1, D // 128)) for m in range(2))
        x1_sel = jnp.where(row16 == k, x1, x1_sel)
        h2_sel = jnp.where(row16 == k, (x1 - mean) * inv * scale[:1] + shift[:1], h2_sel)
        weight = jnp.where(row16 == k, jnp.tile(jax.nn.sigmoid(score), (1, D // 128)), weight)
    h_sel = h2_sel.astype(BF16)
    gate16 = jnp.concatenate([gate_b, gate_b], axis=0)
    base_rows, update_scale = x1_sel + gate16 * h2_sel, gate16 * weight

    def down(f, act):
        return _dot(act, wd_v[f * F_CHUNK:(f + 1) * F_CHUNK, :], _NN)

    y, act = jnp.zeros((16, D), F32), None
    for f in range(F // F_CHUNK):
        gate, up = (_dot(h_sel, w[:, f * F_CHUNK:(f + 1) * F_CHUNK], _NN) for w in (wg_v, wu_v))
        if f > 0:
            y = y + down(f - 1, act)
        act = (gate * jax.nn.sigmoid(gate) * up).astype(BF16)
        if f < T // (2 * LAST_ROWS):
            for k in range(2):
                output_rows(S - T + (2 * f + k) * LAST_ROWS, LAST_ROWS, (gate, up)[k][:8, :1])
        if f == OUT_CHUNK:
            cp_out[1].start()
    routed_rows = base_rows + update_scale * (y + down(F // F_CHUNK - 1, act))

    wait_all(cp_out)
    for k, t in enumerate(routed):
        row = jnp.broadcast_to(routed_rows[k:k + 1], (16, D))
        out_v[t // 16] = jnp.where(row16 == t % 16, row, out_v[t // 16].astype(F32)).astype(BF16)

    fix = [copy(out_v.at[t // 16], out_hbm.at[t // 16]) for t in routed]
    fix[0].start()

    @pl.when(routed[0] // 16 != routed[1] // 16)
    def _():
        fix[1].start()
        fix[1].wait()

    fix[0].wait()


@jax.jit
def pallas_adaLN_cond__linear_kernel_hedgehog__moe_arch_mod__prompt_kernel(
    A_x: jax.Array,
    A_wqkv: jax.Array,
    A_w_phi: jax.Array,
    A_wo: jax.Array,
    B_x: jax.Array,
    B_w_r: jax.Array,
    B_w_gate: jax.Array,
    B_w_up: jax.Array,
    B_w_down: jax.Array,
    c: jax.Array,
    w_mod: jax.Array,
):
    del B_x
    weight_operands = pltpu.VMEM((SG * NOPS, 64, HALF), U32)
    out = pl.pallas_call(
        _kernel,
        out_shape=jax.ShapeDtypeStruct((S // 16, 16, D), BF16),
        in_specs=[pl.BlockSpec(memory_space=pl.ANY)] * 10,
        out_specs=pl.BlockSpec(memory_space=pl.ANY),
        scratch_shapes=[
            pltpu.VMEM((S // 16 + 1, 16, D), BF16),
            pltpu.VMEM((3 * D // 128 + 1, D, 128), BF16),
            pltpu.VMEM((H * DH, DH), BF16),
            pltpu.VMEM((SG + 1, 256, D), BF16),
            pltpu.VMEM((D // 128, 128), BF16),
            pltpu.VMEM((D, F), BF16),
            pltpu.VMEM((D, F), BF16),
            pltpu.VMEM((F, D), BF16),
            pltpu.VMEM((1, D), BF16),
            pltpu.VMEM((6 * D // 128 + 1, D, 128), BF16),
            weight_operands,
            weight_operands,
            weight_operands,
            weight_operands,
            pltpu.VMEM((S // 16, 16, D), BF16),
            pltpu.VMEM((2, 8, D), F32),
            pltpu.VMEM((7, 8, D), F32),
            pltpu.VMEM((4, 128, T), BF16),
            pltpu.VMEM((4, 80, T), BF16),
            pltpu.VMEM((PAIRS, 80, 128), BF16),
            pltpu.VMEM((2, S // 8, 8, 128), F32),
            pltpu.SemaphoreType.DMA((48,)),
            *[pltpu.VMEM((S // 32 + 1, 16, D), F32)] * 2,
            *[pltpu.VMEM((SG, 80, 128), F32)] * 4,
            *[pltpu.VMEM((NOPS, 128, HALF), BF16)] * TILES,
        ],
        compiler_params=pltpu.CompilerParams(vmem_limit_bytes=120 * 1024 * 1024),
        name="hedgehog_moe",
    )(
        A_x.reshape(S // 16, 16, D), A_wqkv, A_w_phi.reshape(H * DH, DH),
        A_wo.reshape(SG, 256, D), B_w_r.reshape(D // 128, 128), B_w_gate, B_w_up, B_w_down, c, w_mod,
    )
    return out.reshape(1, S, D)
```

```python
import functools
import itertools
import math

import jax
import jax.numpy as jnp
from jax import lax
import jax.experimental.pallas as pl
import jax.experimental.pallas.tpu as pltpu

S, D, H, DH, F = 2048, 1024, 32, 32, 3584
PAIRS = H // 2
T = 256
TILES = S // T
SG = 4
UNITS = TILES * SG
HALF = D // 2
F_CHUNK = 512
MOD_CHUNK = 256
LOG2E = math.log2(math.e)
NOPS = 7

KEY_SLOTS = (2, 3, 4, 5)
QUERY_SLOTS = (2, 3, 4, 5)
LN_SLOTS = (1,)
LN_EARLY_SLOTS = (2, 11)
LN_LATE_SLOTS = (13, 3)
LN_SLACK = 4
STORE_SLOT = 6
VALUE_SLOT = 2
FINISH_SLOTS = ((2, 5), (7, 13))
LATE_UNIT = UNITS - 12 if UNITS > 20 else UNITS - 8
EARLY_OUT = max(TILES - 3, 1)
LAST_ROWS = 64
OUT_CHUNK = 2
LEAD1 = 5
PACE = 12
NORM_BACK = 2
LEAD2 = 5
HOLD = 'orqm'

F32 = jnp.float32
BF16 = jnp.bfloat16
U32 = jnp.uint32
I32 = jnp.int32

_NN = (((1,), (0,)), ((), ()))
_NT = (((1,), (1,)), ((), ()))


def _dot(a, b, dims):
    return lax.dot_general(a, b, dims, preferred_element_type=F32)


def _round_bf16(x):
    return x.astype(BF16).astype(F32)


def _bits(x):
    return pltpu.bitcast(x, U32)


def _iota(shape, axis):
    return lax.broadcasted_iota(I32, shape, axis)


def _recip(x):
    return pl.reciprocal(x, full_range=False)


def _join(tokens):
    return functools.reduce(jnp.bitwise_or, tokens)


def _left_operands(a11, a12, a21, a22):
    return a11 + a22, a21 + a22, a11, a22, a11 + a12, a21 - a11, a12 - a22


def _right_operands(b11, b12, b21, b22):
    return b11 + b22, b11, b12 - b22, b21 - b11, b22, b11 + b12, b21 + b22


def _row_sum(x):
    return jnp.sum(x, axis=-1, keepdims=True)


def _inv_std(centered):
    return lax.rsqrt(_row_sum(centered * centered) * (1.0 / D) + 1e-5)


def _row_token(x):
    return _join([_bits(jnp.broadcast_to(x[i], (8, 128))) for i in range(x.shape[0])])


def _transposed_words(x):
    return _bits(x.astype(BF16).T)


def _head_allreduce(x, op):
    r = functools.reduce(op, [x[i:i + 8] for i in range(0, 64, 8)])
    r = op(r, pltpu.roll(r, 4, 0))
    return op(r, pltpu.roll(r, 2, 0))


def _feature_map(p):
    p3 = p.reshape(8, 8, T)
    e_pos = jnp.exp2(p3 - _head_allreduce(p, jnp.maximum)[None])
    e_neg = jnp.exp2(_head_allreduce(p, jnp.minimum)[None] - p3)
    inv_pos, inv_neg = (_recip(_head_allreduce(e.reshape(64, T), jnp.add)) for e in (e_pos, e_neg))
    phi = jnp.concatenate([e_pos * inv_pos[None], e_neg * inv_neg[None]], axis=0)
    token = _bits(inv_pos) | _bits(inv_neg)
    return phi.reshape(128, T).astype(BF16), token[:, :128] | token[:, 128:]


def _kernel(x_hbm, wqkv_hbm, wphi_hbm, wo_hbm, wr_hbm, wg_hbm, wu_hbm, wd_hbm, c_hbm, wmod_hbm,
            out_hbm,
            x_v, wqkv_v, wphi_v, wo_v, wr_v, wg_v, wu_v, wd_v, c_v, wmod_v,
            wq_s, wk_s, wv_s, wo_s, out_v, mod_a, mod_b, phi_s, v_s, kv_s, stat_v,
            sems, *rest):
    x1_v, kv_acc, h_s = rest[:2], rest[2:6], rest[6:]
    sem_ids = itertools.count()

    def copy(src, dst):
        return pltpu.make_async_copy(src, dst, sems.at[next(sem_ids)])

    def copy_slabs(src, dst, first, count):
        sem = sems.at[next(sem_ids)]
        return [pltpu.make_async_copy(src.at[:, pl.ds(k * 128, 128)], dst.at[k], sem)
                for k in range(first, first + count)]

    def wait_all(copies):
        for cp in copies:
            cp.wait()

    def copy_blocks(src, dst, start, size):
        return copy(src.at[pl.ds(start, size)], dst.at[pl.ds(start, size)])

    cp_c, cp_phi, cp_wr = copy(c_hbm, c_v), copy(wphi_hbm, wphi_v), copy(wr_hbm, wr_v)
    cp_x = [copy_blocks(x_hbm, x_v, 16 * i, 16) for i in range(2)]
    cp_x.append(copy_blocks(x_hbm, x_v, 32, S // 16 - 32))
    mod_a_cols = [c0 + l for l in (0, 256) for c0 in range(0, 2 * D, HALF)]
    cp_mod_a = [copy_slabs(wmod_hbm, wmod_v, c0 // 128, 2) for c0 in mod_a_cols]
    cp_wk = [copy_slabs(wqkv_hbm, wqkv_v, 8 + 2 * sg, 2) for sg in range(SG)]
    cp_wv = [copy_slabs(wqkv_hbm, wqkv_v, 16 + 2 * sg, 2) for sg in range(SG)]
    cp_wq = copy_slabs(wqkv_hbm, wqkv_v, 0, 8)
    cp_late = copy_slabs(wmod_hbm, wmod_v, 16, 32) + [cp_wr, copy_blocks(wo_hbm, wo_v, 0, SG)]
    cp_ffn = [copy(wg_hbm, wg_v), copy(wu_hbm, wu_v), copy(wd_hbm, wd_v)]
    cp_out = [copy_blocks(out_v, out_hbm, 0, 16 * EARLY_OUT),
              copy_blocks(out_v, out_hbm, 16 * EARLY_OUT, 16 * (TILES - EARLY_OUT))]
    for cp in (cp_c, cp_x[0], cp_phi, *itertools.chain(*cp_mod_a[:4]), *cp_wk[0],
               *itertools.chain(*cp_mod_a[4:]), *cp_wv[0], *cp_wk[1],
               *cp_wv[1], cp_x[1], *cp_wk[2], *cp_wv[2], *cp_wk[3], *cp_wv[3], cp_x[2], *cp_wq, *cp_late, *cp_ffn):
        cp.start()

    cp_c.wait()
    c = c_v[...].astype(F32)
    silu_c = jnp.broadcast_to(c * jax.nn.sigmoid(c), (16, D)).astype(BF16)
    never = jnp.broadcast_to(c[:, :128] * c[:, :128], (8, 128)) < 0.0
    zero = jnp.max(never.astype(F32)).astype(I32)
    stamps = itertools.count(1)

    def at(i):
        return i + zero * next(stamps)

    def after(words, token):
        head = jnp.concatenate([jnp.where(never, token, words[:8, l:l + 128])
                                for l in range(0, words.shape[1], 128)], axis=1)
        return jnp.concatenate([head, words[8:]], axis=0)

    def hold(ref, token):
        token = pltpu.bitcast(token, ref.dtype)
        ref[ref.shape[0] - 1, :token.shape[0], :128] = token

    def once(value, token):
        return jnp.where(never[:, :1], token, value)

    history, due = [], {}

    def tick(back, step):
        back, step = back - step // 16, step % 16
        return history[-back][8 * step:8 * step + 8, :128]

    def block_product(left, right, dims, tasks):
        assert all(0 <= entry[0] < NOPS for entry in tasks)

        def m(n, slot):
            for at_slot, fn, *slack in tasks:
                if at_slot == slot:
                    due.setdefault(len(history) + sum(slack), []).append(fn())
            tokens = [t for t in due.pop(len(history), []) if t is not None]
            operands = [left(n), right(n)]
            for k, op in enumerate(operands):
                if op.dtype == U32:
                    operands[k] = pltpu.bitcast(after(op, _join(tokens)) if tokens else op, BF16)
            result = _dot(*operands, dims)
            history.append(result)
            return result

        m2, m4 = m(1, 0), m(3, 1)
        c21 = m2 + m4
        m3 = m(2, 2)
        c22 = m3 - m2
        m5 = m(4, 3)
        c12 = m3 + m5
        c11 = m4 - m5
        m1 = m(0, 4)
        c11, c22 = c11 + m1, c22 + m1
        c11 = c11 + m(6, 5)
        c22 = c22 + m(5, 6)
        return c11, c12, c21, c22

    def modulation(col0):
        i, c0 = divmod(col0, D)
        w = jnp.concatenate([wmod_v[at(col0 // 128 + k)] for k in range(2)], axis=1)
        m = _round_bf16(_dot(silu_c, w, _NN)[:8])
        dst, row = (mod_a, i) if i < 2 else (mod_b, i - 2)
        dst[row, :, c0:c0 + MOD_CHUNK] = _round_bf16(1.0 + m) if i % 3 == 1 else m

    def phi_blocks():
        select = (_iota((128, DH), 0) % 64 // 2 == _iota((128, DH), 1)).astype(BF16)
        row = _iota((128, 128), 0)
        same_head = row // 64 * 2 + row % 2 == _iota((128, 128), 1) // DH
        return [jnp.where(same_head, _dot(select, wphi_v[g * 128:(g + 1) * 128, :], _NT), 0.0)
                .astype(BF16) for g in range(D // 128)]

    def fold_phi(col0, dst, sg, l):
        quads = []
        for g in (2 * sg, 2 * sg + 1):
            w = jnp.concatenate([wqkv_v[at(col0 // 128 + g), r:r + 128, :]
                                 for r in (l * 128, HALF + l * 128)], axis=0)
            folded = _dot(phi_bd[g], w, _NT) * LOG2E
            quads += [folded[:, :128], folded[:, 128:]]
        for n, op in enumerate(_left_operands(*quads)):
            dst[sg * NOPS + n, :, l * 128:(l + 1) * 128] = _bits(op.astype(BF16))

    def transpose_wv(sg):
        first, second = (wqkv_v[at(16 + 2 * sg + k)].astype(F32) for k in range(2))
        ops = _left_operands(first[:HALF], first[HALF:], second[:HALF], second[HALF:])
        for n, op in enumerate(ops):
            wv_s[sg * NOPS + n] = _transposed_words(op)

    def split_wo(cp, sg, token):
        hold(wo_v, token)
        w = wo_v[at(sg), :, cp * 256:(cp + 1) * 256].astype(F32)
        ops = _right_operands(w[:128, :128], w[:128, 128:], w[128:, :128], w[128:, 128:])
        for n, op in enumerate(ops):
            wo_s[cp * NOPS + n, :, sg * 128:(sg + 1) * 128] = _transposed_words(op)

    stats = {}

    def load_rows(i, b, n):
        return jnp.concatenate([x_v[pl.ds(at(i * 16 + half * 8 + b), n)].astype(F32)
                                for half in range(2)], axis=0).reshape(4 * n, 8, D)

    def paced(stat, back, step):
        return once(stat, tick(back, step)[None, :, :1]) if back else stat

    def row_statistics(i, b, n):
        mean = _row_sum(load_rows(i, b, n)) * (1.0 / D)
        stats[i, b] = mean, _inv_std(load_rows(i, b, n) - mean)

    def normalize_rows(i, b, n, column_groups, back=0):
        mean, inv = stats[i, b]
        mean = once(mean, inv)
        x = load_rows(i, b, n)
        for l in column_groups:
            m = paced(mean, back, PACE * l)
            lo, hi = (((x[:, :, c0:c0 + 256] - m) * inv * mod_a[at(1), :, c0:c0 + 256][None]
                       + mod_a[at(0), :, c0:c0 + 256][None]).reshape(32 * n, 256)
                      for c0 in (l * 256, HALF + l * 256))
            ops = _right_operands(lo[:16 * n], lo[16 * n:], hi[:16 * n], hi[16 * n:])
            for k, op in enumerate(ops):
                h_s[i][k, 16 * b:16 * (b + n), l * 256:(l + 1) * 256] = op.astype(BF16)

    def layer_norm_rows(i, b, n):
        hold(x_v, tick(LEAD1, 0))
        row_statistics(i, b, n)
        normalize_rows(i, b, n, (0, 1), NORM_BACK)
        return _bits(h_s[i][at(0), 16 * b:16 * (b + 1), :128])

    def project(w_s, sg, i, tasks):
        blocks = block_product(lambda n: w_s[at(sg * NOPS + n)], lambda n: h_s[i][at(n)], _NT, tasks)
        return [[blocks[j // 2 * 2 + half][(j % 2) * 64:(j % 2 + 1) * 64] for half in range(2)]
                for j in range(4)]

    def key_features(p, out):
        phi, token = _feature_map(jnp.concatenate(p, axis=1))
        out.append(phi)
        return token

    def store_values(v):
        for j in range(4):
            v_s[j, :64, :] = jnp.concatenate(v[j], axis=1).astype(BF16)
        return _bits(v_s[at(0), :16, :128])

    def accumulate_kv(sg, i, phi):
        for j in range(4):
            kv = _dot(v_s[at(j)], phi[j], _NT)
            kv = kv if i == 0 else kv_acc[j][at(sg)] + kv
            if i + 1 < TILES:
                kv_acc[j][sg] = kv
            else:
                row = _iota((80, 128), 0)
                head = jnp.where(row < 64, row // DH, row // 8 % 2)
                kv_s[4 * sg + j] = jnp.where(head == _iota((80, 128), 1) % 2, kv, 0.0).astype(BF16)

    v_s[:, 64:, :] = jnp.ones((4, 16, T), BF16)

    cp_x[0].wait()
    for b in range(0, 8, 2):
        row_statistics(0, b, 2)
    cp_phi.wait()
    phi_bd = phi_blocks()
    for l in range(2):
        for k in range(4 * l, 4 * l + 4):
            wait_all(cp_mod_a[k])
            modulation(mod_a_cols[k])
        for b in range(0, 8, 2):
            normalize_rows(0, b, 2, (l,))
        if l == 0:
            wait_all(cp_wk[0])
            for k in range(HALF // 128):
                fold_phi(D, wk_s, 0, k)
    wait_all(cp_wv[0])

    task = functools.partial
    pending = None
    for u in range(UNITS):
        i, sg = divmod(u, SG)
        if 0 < u < SG:
            wait_all(cp_wk[sg] + cp_wv[sg] + cp_x[1:2] * (sg == 2))
            for l in range(HALF // 128):
                fold_phi(D, wk_s, sg, l)
        if u == SG + 2:
            cp_x[2].wait()
        if u == LATE_UNIT:
            wait_all(cp_late)
            wait_all(cp_wq)
        if LATE_UNIT <= u < LATE_UNIT + 8:
            k = 2 * (u - LATE_UNIT)
            if 'q' in HOLD:
                hold(wqkv_v, _bits(pk[0][1][:8]))
            fold_phi(0, wq_s, *divmod(k, 4))
            fold_phi(0, wq_s, *divmod(k + 1, 4))

        first, last = [], []
        if i < 2:
            work = zip(LN_EARLY_SLOTS, (4 * sg - 8, 4 * sg - 6), (2, 2)) if sg >= 2 else ()
        elif i + 1 < TILES:
            slots = LN_LATE_SLOTS if u >= LATE_UNIT else LN_SLOTS
            work = [(slot, 2 * sg + k, 2 // len(slots)) for k, slot in enumerate(slots)]
        else:
            work = ()
        for slot, b, n in work:
            (first if slot < 7 else last).append(
                (slot % 7, task(layer_norm_rows, i + 1, b, n), 3 if i < 2 else 2 + n))
        if pending is not None:
            first.append((VALUE_SLOT, task(store_values, pending[0])))
        pk = project(wk_s, sg, i, first)
        if i == 0:
            transpose_wv(sg)
        if pending is not None:
            accumulate_kv(*pending[1:])
        phi = []
        last += [(KEY_SLOTS[j], task(key_features, pk[j], phi)) for j in range(4)]
        if i == TILES - 1:
            last += [(2 + k, task(split_wo, sg, k, _bits(pk[k][0][:8]))) for k in range(4)]
        pending = (project(wv_s, sg, i, last), sg, i, phi)
    store_values(pending[0])
    accumulate_kv(*pending[1:])

    def output_vectors():
        wr = wr_v[...].astype(F32)
        wr = jnp.concatenate([jnp.broadcast_to(wr[l:l + 1, :], (8, 128)) for l in range(D // 128)], axis=1)
        shift, scale, gate_b = mod_b[1], mod_b[2], mod_b[3]
        mod_b[4] = scale * wr
        mod_b[5] = scale * gate_b
        mod_b[6] = shift * gate_b
        return _row_sum(shift * wr)

    def query_features(p, out):
        phi, token = _feature_map(jnp.concatenate(p, axis=1))
        out.append(phi)
        return token

    def attend(feats, sg, out):
        out.extend(_dot(kv_s[at(4 * sg + j)], feats[j], _NN) for j in range(4))

    o_parts, o_ops = {}, {}

    def o_operand(i, n):
        if (i, n) not in o_ops:
            o_ops[i, n] = jnp.concatenate([o_parts[i, sg][n] for sg in range(SG)], axis=1).astype(BF16)
        return o_ops[i, n]

    def store_attention(nums, sg, i):
        blocks = []
        for num in nums:
            num = num.reshape(10, 8, T)
            inv = _recip(num[8:] + 1e-6)
            o = jnp.concatenate([num[:4] * inv[0:1], num[4:8] * inv[1:2]], axis=0)
            blocks.append(o.reshape(64, T))
        first = jnp.concatenate(blocks[:2], axis=0).T
        second = jnp.concatenate(blocks[2:], axis=0).T
        quads = first[:128], second[:128], first[128:], second[128:]
        o_parts[i, sg] = _left_operands(*quads)
        return _join([_bits(q[120:]) for q in quads])

    def project_out(i, cp, tasks):
        return block_product(lambda n: o_operand(i, n), lambda n: wo_s[at(cp * NOPS + n)], _NT, tasks)

    def add_residual(blocks, i, cp):
        for k in (2, 1, 0, 3):
            attn = blocks[k]
            if 'r' in HOLD:
                hold(x_v, _bits(attn[:8]))
            cs = pl.ds(cp * 256 + (k % 2) * 128, 128)
            x = x_v[pl.ds(at(i * 16 + (k // 2) * 8), 8), :, cs].astype(F32).reshape(16, 8, 128)
            x1 = x + mod_b[at(0), :, cs][None] * attn.reshape(16, 8, 128)
            x1_v[i % 2][pl.ds(i // 2 * 16 + (k // 2) * 8, 8), :, cs] = x1.reshape(8, 16, 128)

    top = [jnp.full((8, 128), -jnp.inf, F32), jnp.zeros((8, 128), I32)] * 2

    def load_attended(r0, n):
        i = r0 // T
        return x1_v[i % 2][pl.ds(at(i // 2 * 16 + r0 % T // 16), n // 16)].reshape(n // 8, 8, D)

    def mean_attended(r0, n):
        if r0 < S - T and LEAD2:
            hold(x1_v[r0 // T % 2], tick(LEAD2, 0))
        stats[r0] = _row_sum(load_attended(r0, n)) * (1.0 / D)
        return _row_token(stats[r0])

    def score_rows(r0, n):
        mean = stats.pop(r0)
        centered = load_attended(r0, n) - mean
        routed = _row_sum(centered * mod_b[at(4)][None])
        inv = _inv_std(centered)
        for k, stat in enumerate((mean, inv)):
            stat_v[k, pl.ds(r0 // 8, n // 8)] = jnp.broadcast_to(stat, (n // 8, 8, 128))
        stats[r0] = mean, inv
        score = _round_bf16(routed * inv + score_bias)
        best, best_i, second, second_i = top
        for b in range(n // 8):
            s, t = jnp.broadcast_to(score[b], (8, 128)), _iota((8, 128), 0) + (r0 + 8 * b)
            above_best, above_second = s > best, s > second
            second = jnp.where(above_best, best, jnp.where(above_second, s, second))
            second_i = jnp.where(above_best, best_i, jnp.where(above_second, t, second_i))
            best = jnp.where(above_best, s, best)
            best_i = jnp.where(above_best, t, best_i)
        top[:] = best, best_i, second, second_i

    def output_rows(r0, n, token=None):
        mean, inv = stats.pop(r0)
        if token is not None:
            inv = once(inv, token[None])
        x1 = load_attended(r0, n)
        out = x1 + ((x1 - once(mean, inv)) * inv * mod_b[at(5)][None] + mod_b[at(6)][None])
        out_v[pl.ds(r0 // 16, n // 16)] = out.reshape(n // 16, 16, D).astype(BF16)

    def finish_rows(r0, n):
        score_rows(r0, n)
        output_rows(r0, n)
        return _bits(top[3]) | _bits(out_v[at(0), :, :128])

    def run(tasks):
        for _, fn, *_ in sorted(tasks, key=lambda item: item[0]):
            fn()

    feats = attn = None
    for u in range(UNITS + SG):
        first, last = [], []
        if feats is not None:
            tile, sg = divmod(u - 1, SG)
            nums = []
            first.append((0, task(attend, feats, sg, nums)))
            first.append((STORE_SLOT, task(store_attention, nums, sg, tile)))
        if attn is not None:
            add_residual(attn, *divmod(u - SG - 1, SG))
        if u >= 2 * SG:
            for k, slots in enumerate(FINISH_SLOTS):
                n = 64 // len(FINISH_SLOTS)
                r0 = (u - 2 * SG) * 64 + n * k
                for slot, fn in zip(slots, (mean_attended, finish_rows)):
                    if u >= UNITS:
                        last.append((slot // 2, task(fn, r0, n)))
                    else:
                        (first if slot < 7 else last).append((slot % 7, task(fn, r0, n)))
        feats = attn = None
        if u < UNITS:
            tile, sg = divmod(u, SG)
            pq = project(wq_s, sg, tile, first)
            feats = []
            last += [(QUERY_SLOTS[j], task(query_features, pq[j], feats)) for j in range(4)]
        else:
            run(first)
        if u >= SG:
            attn = project_out(*divmod(u - SG, SG), last)
        else:
            run(last)
            for k in range(4):
                modulation(2 * D + (4 * u + k) * MOD_CHUNK)
            if u == SG - 1:
                score_bias = output_vectors()
        if u == (EARLY_OUT + 2) * SG - 1:
            cp_out[0].start()
            wait_all(cp_ffn)
    add_residual(attn, TILES - 1, SG - 1)
    for fn in (mean_attended, score_rows):
        for r0 in range(S - T, S, LAST_ROWS):
            fn(r0, LAST_ROWS)
    best, best_i, second, second_i = top

    scores = jnp.concatenate([best, second], axis=0)
    tokens = jnp.concatenate([best_i, second_i], axis=0)

    def take_top(scores):
        top = jnp.max(scores, axis=0, keepdims=True)
        tok = jnp.min(jnp.where(scores == top, tokens, S - 1).astype(F32), axis=0, keepdims=True)
        return top, tok.astype(I32)

    score0, tok0 = take_top(scores)
    score1, tok1 = take_top(jnp.where(tokens == tok0, -jnp.inf, scores))
    routed = [jnp.clip(tok[0, 0], 0, S - 1) for tok in (tok0, tok1)]

    row16 = _iota((16, D), 0)
    shift, scale, gate_b = mod_b[at(1)], mod_b[at(2)], mod_b[at(3)]
    x1_sel = h2_sel = weight = jnp.zeros((16, D), F32)
    for k, (t, score) in enumerate(zip(routed, (score0, score1))):
        blk, row = t // (2 * T) * 16 + t % T // 16, pl.ds(t % 16, 1)
        x1 = jnp.where(t // T % 2 == 0, x1_v[0][blk, row, :], x1_v[1][blk, row, :])
        mean, inv = (jnp.tile(stat_v[m, t // 8, pl.ds(t % 8, 1), :], (1, D // 128)) for m in range(2))
        x1_sel = jnp.where(row16 == k, x1, x1_sel)
        h2_sel = jnp.where(row16 == k, (x1 - mean) * inv * scale[:1] + shift[:1], h2_sel)
        weight = jnp.where(row16 == k, jnp.tile(jax.nn.sigmoid(score), (1, D // 128)), weight)
    h_sel = h2_sel.astype(BF16)
    gate16 = jnp.concatenate([gate_b, gate_b], axis=0)
    base_rows, update_scale = x1_sel + gate16 * h2_sel, gate16 * weight

    def down(f, act):
        return _dot(act, wd_v[f * F_CHUNK:(f + 1) * F_CHUNK, :], _NN)

    y, act = jnp.zeros((16, D), F32), None
    for f in range(F // F_CHUNK):
        gate, up = (_dot(h_sel, w[:, f * F_CHUNK:(f + 1) * F_CHUNK], _NN) for w in (wg_v, wu_v))
        if f > 0:
            y = y + down(f - 1, act)
        act = (gate * jax.nn.sigmoid(gate) * up).astype(BF16)
        if f < T // (2 * LAST_ROWS):
            for k in range(2):
                output_rows(S - T + (2 * f + k) * LAST_ROWS, LAST_ROWS, (gate, up)[k][:8, :1])
        if f == OUT_CHUNK:
            cp_out[1].start()
    routed_rows = base_rows + update_scale * (y + down(F // F_CHUNK - 1, act))

    wait_all(cp_out)
    for k, t in enumerate(routed):
        row = jnp.broadcast_to(routed_rows[k:k + 1], (16, D))
        out_v[t // 16] = jnp.where(row16 == t % 16, row, out_v[t // 16].astype(F32)).astype(BF16)

    fix = [copy(out_v.at[t // 16], out_hbm.at[t // 16]) for t in routed]
    fix[0].start()

    @pl.when(routed[0] // 16 != routed[1] // 16)
    def _():
        fix[1].start()
        fix[1].wait()

    fix[0].wait()


@jax.jit
def pallas_adaLN_cond__linear_kernel_hedgehog__moe_arch_mod__prompt_kernel(
    A_x: jax.Array,
    A_wqkv: jax.Array,
    A_w_phi: jax.Array,
    A_wo: jax.Array,
    B_x: jax.Array,
    B_w_r: jax.Array,
    B_w_gate: jax.Array,
    B_w_up: jax.Array,
    B_w_down: jax.Array,
    c: jax.Array,
    w_mod: jax.Array,
):
    del B_x
    weight_operands = pltpu.VMEM((SG * NOPS, 64, HALF), U32)
    out = pl.pallas_call(
        _kernel,
        out_shape=jax.ShapeDtypeStruct((S // 16, 16, D), BF16),
        in_specs=[pl.BlockSpec(memory_space=pl.ANY)] * 10,
        out_specs=pl.BlockSpec(memory_space=pl.ANY),
        scratch_shapes=[
            pltpu.VMEM((S // 16 + 1, 16, D), BF16),
            pltpu.VMEM((3 * D // 128 + 1, D, 128), BF16),
            pltpu.VMEM((H * DH, DH), BF16),
            pltpu.VMEM((SG + 1, 256, D), BF16),
            pltpu.VMEM((D // 128, 128), BF16),
            pltpu.VMEM((D, F), BF16),
            pltpu.VMEM((D, F), BF16),
            pltpu.VMEM((F, D), BF16),
            pltpu.VMEM((1, D), BF16),
            pltpu.VMEM((6 * D // 128 + 1, D, 128), BF16),
            weight_operands,
            weight_operands,
            weight_operands,
            weight_operands,
            pltpu.VMEM((S // 16, 16, D), BF16),
            pltpu.VMEM((2, 8, D), F32),
            pltpu.VMEM((7, 8, D), F32),
            pltpu.VMEM((4, 128, T), BF16),
            pltpu.VMEM((4, 80, T), BF16),
            pltpu.VMEM((PAIRS, 80, 128), BF16),
            pltpu.VMEM((2, S // 8, 8, 128), F32),
            pltpu.SemaphoreType.DMA((48,)),
            *[pltpu.VMEM((S // 32 + 1, 16, D), F32)] * 2,
            *[pltpu.VMEM((SG, 80, 128), F32)] * 4,
            *[pltpu.VMEM((NOPS, 128, HALF), BF16)] * TILES,
        ],
        compiler_params=pltpu.CompilerParams(vmem_limit_bytes=120 * 1024 * 1024),
        name="hedgehog_moe",
    )(
        A_x.reshape(S // 16, 16, D), A_wqkv, A_w_phi.reshape(H * DH, DH),
        A_wo.reshape(SG, 256, D), B_w_r.reshape(D // 128, 128), B_w_gate, B_w_up, B_w_down, c, w_mod,
    )
    return out.reshape(1, S, D)
```

```python
import functools
import itertools
import math

import jax
import jax.numpy as jnp
from jax import lax
import jax.experimental.pallas as pl
import jax.experimental.pallas.tpu as pltpu

S, D, H, DH, F = 2048, 1024, 32, 32, 3584
T = 256
TILES = S // T
GROUPS = 4
UNITS = TILES * GROUPS
HALF = D // 2
NOPS = 7
F_CHUNK = 512
LOG2E = math.log2(math.e)

KEY_SLOTS = (9, 10, 11, 12)
NORM_SLOTS = (1,)
NORM_SLOTS_EARLY = (2, 11)
NORM_SLOTS_LATE = (13, 3)
NORM_RELEASE = 5
NORM_PACE = 12
QUERY_SLOTS = (9, 10, 11, 12)
TRANSPOSE_SLOT = 6
FINISH_SLOTS = ((2, 5), (7, 13))
FINISH_RELEASE = 5
LATE_UNIT = UNITS - 12 if UNITS > 20 else UNITS - 8
EARLY_TILES = max(TILES - 3, 1)
LAST_ROWS = 64

F32 = jnp.float32
BF16 = jnp.bfloat16
U32 = jnp.uint32
I32 = jnp.int32

_NN = (((1,), (0,)), ((), ()))
_NT = (((1,), (1,)), ((), ()))


def _dot(a, b, dims):
    return lax.dot_general(a, b, dims, preferred_element_type=F32)


def _round_bf16(x):
    return x.astype(BF16).astype(F32)


def _bits(x):
    return pltpu.bitcast(x, U32)


def _bf16(words):
    return pltpu.bitcast(words, BF16)


def _iota(shape, axis):
    return lax.broadcasted_iota(I32, shape, axis)


def _recip(x):
    return pl.reciprocal(x, full_range=False)


def _join(tokens):
    return functools.reduce(jnp.bitwise_or, tokens)


def _left_operands(a11, a12, a21, a22):
    return a11 + a22, a21 + a22, a11, a22, a11 + a12, a21 - a11, a12 - a22


def _right_operands(b11, b12, b21, b22):
    return b11 + b22, b11, b12 - b22, b21 - b11, b22, b11 + b12, b21 + b22


def _row_sum(x):
    return jnp.sum(x, axis=-1, keepdims=True)


def _inv_std(centered):
    return lax.rsqrt(_row_sum(centered * centered) * (1.0 / D) + 1e-5)


def _head_allreduce(x, op):
    r = functools.reduce(op, [x[i:i + 8] for i in range(0, 64, 8)])
    r = op(r, pltpu.roll(r, 4, 0))
    return op(r, pltpu.roll(r, 2, 0))


def _feature_map(p):
    p3 = p.reshape(8, 8, T)
    e_pos = jnp.exp2(p3 - _head_allreduce(p, jnp.maximum)[None])
    e_neg = jnp.exp2(_head_allreduce(p, jnp.minimum)[None] - p3)
    inv_pos, inv_neg = (_recip(_head_allreduce(e.reshape(64, T), jnp.add)) for e in (e_pos, e_neg))
    phi = jnp.concatenate([e_pos * inv_pos[None], e_neg * inv_neg[None]], axis=0)
    token = _bits(inv_pos) | _bits(inv_neg)
    return phi.reshape(2 * 64, T).astype(BF16), token[:, :128] | token[:, 128:]


def _kernel(x_hbm, wqkv_hbm, wphi_hbm, wo_hbm, wr_hbm, wg_hbm, wu_hbm, wd_hbm, c_hbm, wmod_hbm,
            out_hbm,
            x_v, wqkv_v, wphi_v, wo_v, wr_v, wg_v, wu_v, wd_v, c_v, wmod_v,
            wq_s, wk_s, wv_s, wo_s, out_v, mod_a, mod_b, kv_s, stat_v,
            sems, *rest):
    x1_v, kv_acc, h_s = rest[:2], rest[2:6], rest[6:]
    task = functools.partial

    sem_ids = itertools.count()

    def copy(src, dst):
        return pltpu.make_async_copy(src, dst, sems.at[next(sem_ids)])

    def copy_blocks(src, dst, start, stop):
        return copy(src.at[pl.ds(start, stop - start)], dst.at[pl.ds(start, stop - start)])

    def copy_slabs(src, dst, first, count):
        sem = sems.at[next(sem_ids)]
        return [pltpu.make_async_copy(src.at[:, pl.ds(k * 128, 128)], dst.at[k], sem)
                for k in range(first, first + count)]

    def wait_all(copies):
        for cp in copies:
            cp.wait()

    mod_a_cols = [c0 + l for l in (0, 256) for c0 in range(0, 2 * D, HALF)]
    cp_c, cp_phi, cp_wr = copy(c_hbm, c_v), copy(wphi_hbm, wphi_v), copy(wr_hbm, wr_v)
    cp_x = [copy_blocks(x_hbm, x_v, *span) for span in ((0, 16), (16, 32), (32, S // 16))]
    cp_mod_a = [copy_slabs(wmod_hbm, wmod_v, c0 // 128, 2) for c0 in mod_a_cols]
    cp_wk = [copy_slabs(wqkv_hbm, wqkv_v, 8 + 2 * g, 2) for g in range(GROUPS)]
    cp_wv = [copy_slabs(wqkv_hbm, wqkv_v, 16 + 2 * g, 2) for g in range(GROUPS)]
    cp_late = (copy_slabs(wqkv_hbm, wqkv_v, 0, 8) + copy_slabs(wmod_hbm, wmod_v, 16, 32)
               + [cp_wr, copy_blocks(wo_hbm, wo_v, 0, GROUPS)])
    cp_ffn = [copy(wg_hbm, wg_v), copy(wu_hbm, wu_v), copy(wd_hbm, wd_v)]
    cp_out = [copy_blocks(out_v, out_hbm, 16 * first, 16 * stop) for first, stop in
              ((0, EARLY_TILES), (EARLY_TILES, TILES - 1), (TILES - 1, TILES))]
    for cp in (cp_c, cp_x[0], cp_phi, *itertools.chain(*cp_mod_a[:4]), *cp_wk[0],
               *itertools.chain(*cp_mod_a[4:]), *cp_wv[0], *cp_wk[1], *cp_wv[1], cp_x[1],
               *cp_wk[2], *cp_wv[2], *cp_wk[3], *cp_wv[3], cp_x[2], *cp_late, *cp_ffn):
        cp.start()

    cp_c.wait()
    c = c_v[...].astype(F32)
    silu_c = jnp.broadcast_to(c * jax.nn.sigmoid(c), (16, D)).astype(BF16)

    never = jnp.broadcast_to(c[:, :128] * c[:, :128], (8, 128)) < 0.0
    zero = jnp.max(never.astype(F32)).astype(I32)
    stamps = itertools.count(1)
    history, due = [], {}

    def at(i):
        return i + zero * next(stamps)

    def after(words, token):
        head = jnp.concatenate([jnp.where(never, token, words[:8, l:l + 128])
                                for l in range(0, words.shape[1], 128)], axis=1)
        return jnp.concatenate([head, words[8:]], axis=0)

    def hold(ref, token):
        token = pltpu.bitcast(token, ref.dtype)
        ref[ref.shape[0] - 1, :token.shape[0], :128] = token

    def once(stat, token):
        return jnp.where(never[:, :1], token, stat)

    def tick(back, step=0):
        back, step = back - step // 16, step % 16
        return history[-back][8 * step:8 * step + 8, :128]

    def block_product(left, right, tasks):
        assert all(0 <= entry[0] < NOPS for entry in tasks)

        def m(n, slot):
            for at_slot, fn, *slack in tasks:
                if at_slot == slot:
                    due.setdefault(len(history) + sum(slack), []).append(fn())
            tokens = [t for t in due.pop(len(history), []) if t is not None]
            operands = [left(n), right(n)]
            for k, op in enumerate(operands):
                if op.dtype == U32:
                    operands[k] = _bf16(after(op, _join(tokens)) if tokens else op)
                    tokens = []
            history.append(_dot(*operands, _NT))
            return history[-1]

        m2, m4 = m(1, 0), m(3, 1)
        c21 = m2 + m4
        m3 = m(2, 2)
        c22 = m3 - m2
        m5 = m(4, 3)
        c12 = m3 + m5
        c11 = m4 - m5
        m1 = m(0, 4)
        c11, c22 = c11 + m1, c22 + m1
        c11 = c11 + m(6, 5)
        c22 = c22 + m(5, 6)
        return c11, c12, c21, c22

    def split_tasks(tasks):
        return ([t for t in tasks if t[0] < NOPS],
                [(t[0] - NOPS, *t[1:]) for t in tasks if t[0] >= NOPS])

    def modulation(col0):
        i, c0 = divmod(col0, D)
        w = jnp.concatenate([wmod_v[at(col0 // 128 + k)] for k in range(2)], axis=1)
        m = _round_bf16(_dot(silu_c, w, _NN)[:8])
        dst, row = (mod_a, i) if i < 2 else (mod_b, i - 2)
        dst[row, :, c0:c0 + 256] = _round_bf16(1.0 + m) if i % 3 == 1 else m

    def phi_blocks():
        select = (_iota((128, DH), 0) % 64 // 2 == _iota((128, DH), 1)).astype(BF16)
        row = _iota((128, 128), 0)
        same_head = row // 64 * 2 + row % 2 == _iota((128, 128), 1) // DH
        return [jnp.where(same_head, _dot(select, wphi_v[k * 128:(k + 1) * 128, :], _NT), 0.0)
                .astype(BF16) for k in range(D // 128)]

    def fold_phi(col0, dst, g, l):
        quads = []
        for k in (2 * g, 2 * g + 1):
            w = jnp.concatenate([wqkv_v[at(col0 // 128 + k), r:r + 128, :]
                                 for r in (l * 128, HALF + l * 128)], axis=0)
            folded = _dot(phi_bd[k], w, _NT) * LOG2E
            quads += [folded[:, :128], folded[:, 128:]]
        for n, op in enumerate(_left_operands(*quads)):
            dst[g * NOPS + n, :, l * 128:(l + 1) * 128] = _bits(op.astype(BF16))

    def transpose_wv(g):
        first, second = (wqkv_v[at(16 + 2 * g + k)].astype(F32) for k in range(2))
        ops = _left_operands(first[:HALF], first[HALF:], second[:HALF], second[HALF:])
        for n, op in enumerate(ops):
            wv_s[g * NOPS + n] = _bits(op.astype(BF16).T)

    def transpose_wo(cols, g):
        hold(wo_v, tick(1))
        w = wo_v[at(g), :, cols * 256:(cols + 1) * 256].astype(F32)
        ops = _right_operands(w[:128, :128], w[:128, 128:], w[128:, :128], w[128:, 128:])
        for n, op in enumerate(ops):
            wo_s[cols * NOPS + n, :, g * 128:(g + 1) * 128] = _bits(op.astype(BF16).T)

    stats = {}

    def load_rows(i, b, n):
        return jnp.concatenate([x_v[pl.ds(at(i * 16 + half * 8 + b), n)].astype(F32)
                                for half in range(2)], axis=0).reshape(4 * n, 8, D)

    def row_statistics(i, b, n):
        mean = _row_sum(load_rows(i, b, n)) * (1.0 / D)
        stats[i, b] = mean, _inv_std(load_rows(i, b, n) - mean)

    def normalize_rows(i, b, n, column_groups, back=0):
        mean, inv = stats[i, b]
        mean = once(mean, inv)
        x = load_rows(i, b, n)
        for l in column_groups:
            m = once(mean, tick(back, NORM_PACE * l)[None, :, :1]) if back else mean
            lo, hi = (((x[:, :, c0:c0 + 256] - m) * inv * mod_a[at(1), :, c0:c0 + 256][None]
                       + mod_a[at(0), :, c0:c0 + 256][None]).reshape(32 * n, 256)
                      for c0 in (l * 256, HALF + l * 256))
            ops = _right_operands(lo[:16 * n], lo[16 * n:], hi[:16 * n], hi[16 * n:])
            for k, op in enumerate(ops):
                h_s[i][k, 8 * b:8 * (b + n), l * 256:(l + 1) * 256] = _bits(op.astype(BF16))

    def layer_norm_rows(i, b, n):
        hold(x_v, tick(NORM_RELEASE))
        row_statistics(i, b, n)
        normalize_rows(i, b, n, (0, 1), back=2)
        return h_s[i][at(0), 8 * b:8 * (b + 1), :128]

    def project(w_s, g, i, tasks):
        blocks = block_product(lambda n: w_s[at(g * NOPS + n)], lambda n: h_s[i][at(n)], tasks)
        return [jnp.concatenate([blocks[j // 2 * 2 + half][j % 2 * 64:(j % 2 + 1) * 64]
                                 for half in range(2)], axis=1) for j in range(4)]

    def features(p, out):
        phi, token = _feature_map(p)
        out.append(phi)
        return token

    def accumulate_kv(v, phi, g, i):
        for j in range(4):
            values = jnp.concatenate([v[j], jnp.ones((16, T), F32)], axis=0).astype(BF16)
            kv = _dot(values, phi[j], _NT)
            kv = kv if i == 0 else kv_acc[j][at(g)] + kv
            if i + 1 < TILES:
                kv_acc[j][g] = kv
            else:
                row = _iota((80, 128), 0)
                head = jnp.where(row < 64, row // DH, row // 8 % 2)
                kv_s[4 * g + j] = _bits(
                    jnp.where(head == _iota((80, 128), 1) % 2, kv, 0.0).astype(BF16))

    cp_x[0].wait()
    for b in range(0, 8, 2):
        row_statistics(0, b, 2)
    cp_phi.wait()
    phi_bd = phi_blocks()
    for l in range(2):
        for k in range(4 * l, 4 * l + 4):
            wait_all(cp_mod_a[k])
            modulation(mod_a_cols[k])
        for b in range(0, 8, 2):
            normalize_rows(0, b, 2, (l,))
        if l == 0:
            wait_all(cp_wk[0])
            for k in range(HALF // 128):
                fold_phi(D, wk_s, 0, k)
    wait_all(cp_wv[0])

    pending = None
    for u in range(UNITS):
        i, g = divmod(u, GROUPS)
        if 0 < u < GROUPS:
            wait_all(cp_wk[g] + cp_wv[g] + cp_x[1:2] * (g == 2))
            for l in range(HALF // 128):
                fold_phi(D, wk_s, g, l)
        if u == GROUPS + 2:
            cp_x[2].wait()
        if u == LATE_UNIT:
            wait_all(cp_late)
        if LATE_UNIT <= u < LATE_UNIT + 8:
            hold(wqkv_v, tick(13))
            for k in range(2 * (u - LATE_UNIT), 2 * (u - LATE_UNIT + 1)):
                fold_phi(0, wq_s, *divmod(k, HALF // 128))

        if i < 2:
            work = zip(NORM_SLOTS_EARLY, (4 * g - 8, 4 * g - 6), (2, 2), (3, 3)) if g >= 2 else ()
        elif i + 1 < TILES:
            slots = NORM_SLOTS_LATE if u >= LATE_UNIT else NORM_SLOTS
            n = 2 // len(slots)
            work = [(slot, 2 * g + k, n, 2 + n) for k, slot in enumerate(slots)]
        else:
            work = ()
        first, last = split_tasks([(slot, task(layer_norm_rows, i + 1, b, n), slack)
                                   for slot, b, n, slack in work])
        pk = project(wk_s, g, i, first)
        if i == 0:
            transpose_wv(g)
        if pending is not None:
            accumulate_kv(*pending)
        phi = []
        last += [(KEY_SLOTS[j] - NOPS, task(features, pk[j], phi)) for j in range(4)]
        if i == TILES - 1:
            last += [(3 + k, task(transpose_wo, g, k)) for k in range(GROUPS)]
        pending = project(wv_s, g, i, last), phi, g, i
    accumulate_kv(*pending)

    o_parts, o_ops = {}, {}
    top = [jnp.full((8, 128), -jnp.inf, F32), jnp.zeros((8, 128), I32)] * 2

    def output_vectors():
        wr = wr_v[...].astype(F32)
        wr = jnp.concatenate([jnp.broadcast_to(wr[l:l + 1], (8, 128)) for l in range(D // 128)], axis=1)
        shift, scale, gate = mod_b[1], mod_b[2], mod_b[3]
        mod_b[4] = scale * wr
        mod_b[5] = scale * gate
        mod_b[6] = shift * gate
        return _row_sum(shift * wr)

    def attend(phi, g, out):
        out.extend(_dot(_bf16(kv_s[at(4 * g + j)]), phi[j], _NN) for j in range(4))

    def transpose_attention(nums, i, g):
        blocks = []
        for num in nums:
            num = num.reshape(10, 8, T)
            inv = _recip(num[8:] + 1e-6)
            o = jnp.concatenate([num[:4] * inv[0:1], num[4:8] * inv[1:2]], axis=0)
            blocks.append(o.reshape(64, T))
        first = jnp.concatenate(blocks[:2], axis=0).T
        second = jnp.concatenate(blocks[2:], axis=0).T
        quads = first[:128], second[:128], first[128:], second[128:]
        o_parts[i, g] = _left_operands(*quads)
        return _join([_bits(q[120:]) for q in quads])

    def attention_operand(i, n):
        if (i, n) not in o_ops:
            parts = [o_parts[i, g][n] for g in range(GROUPS)]
            o_ops[i, n] = jnp.concatenate(parts, axis=1).astype(BF16)
        return o_ops[i, n]

    def add_residual(blocks, i, cols):
        for k in (2, 1, 0, 3):
            hold(x_v, blocks[k][:8])
            cs = pl.ds(cols * 256 + k % 2 * 128, 128)
            x = x_v[pl.ds(at(i * 16 + k // 2 * 8), 8), :, cs].astype(F32).reshape(16, 8, 128)
            x1 = x + mod_b[at(0), :, cs][None] * blocks[k].reshape(16, 8, 128)
            x1_v[i % 2][pl.ds(i // 2 * 16 + k // 2 * 8, 8), :, cs] = x1.reshape(8, 16, 128)

    def load_attended(r0, n):
        i = r0 // T
        return x1_v[i % 2][pl.ds(at(i // 2 * 16 + r0 % T // 16), n // 16)].reshape(n // 8, 8, D)

    def mean_attended(r0, n):
        if r0 < S - T:
            hold(x1_v[r0 // T % 2], tick(FINISH_RELEASE))
        stats[r0] = _row_sum(load_attended(r0, n)) * (1.0 / D)
        return _join([_bits(jnp.broadcast_to(stats[r0][k], (8, 128))) for k in range(n // 8)])

    def score_rows(r0, n):
        mean = stats[r0]
        centered = load_attended(r0, n) - mean
        routed = _row_sum(centered * mod_b[at(4)][None])
        inv = _inv_std(centered)
        for k, stat in enumerate((mean, inv)):
            stat_v[k, pl.ds(r0 // 8, n // 8)] = jnp.broadcast_to(stat, (n // 8, 8, 128))
        stats[r0] = mean, inv
        score = _round_bf16(routed * inv + score_bias)
        best, best_i, second, second_i = top
        for b in range(n // 8):
            s, t = jnp.broadcast_to(score[b], (8, 128)), _iota((8, 128), 0) + (r0 + 8 * b)
            above_best, above_second = s > best, s > second
            second = jnp.where(above_best, best, jnp.where(above_second, s, second))
            second_i = jnp.where(above_best, best_i, jnp.where(above_second, t, second_i))
            best = jnp.where(above_best, s, best)
            best_i = jnp.where(above_best, t, best_i)
        top[:] = best, best_i, second, second_i

    def output_rows(r0, n, token=None):
        mean, inv = stats[r0]
        if token is not None:
            inv = once(inv, token[None])
        x1 = load_attended(r0, n)
        out = x1 + ((x1 - once(mean, inv)) * inv * mod_b[at(5)][None] + mod_b[at(6)][None])
        out_v[pl.ds(r0 // 16, n // 16)] = out.reshape(n // 16, 16, D).astype(BF16)

    def finish_rows(r0, n):
        score_rows(r0, n)
        output_rows(r0, n)
        return _bits(top[3]) | _bits(out_v[at(0), :, :128])

    phi = attn = None
    for u in range(UNITS + GROUPS):
        tasks = []
        if phi is not None:
            nums = []
            tasks += [(0, task(attend, phi, (u - 1) % GROUPS, nums)),
                      (TRANSPOSE_SLOT, task(transpose_attention, nums, *divmod(u - 1, GROUPS)))]
        if attn is not None:
            add_residual(attn, *divmod(u - GROUPS - 1, GROUPS))
        if u >= 2 * GROUPS:
            n = 64 // len(FINISH_SLOTS)
            for k, slots in enumerate(FINISH_SLOTS):
                for slot, fn in zip(slots, (mean_attended, finish_rows)):
                    tasks.append((slot if u < UNITS else NOPS + slot // 2,
                                  task(fn, (u - 2 * GROUPS) * 64 + n * k, n)))
        first, last = split_tasks(tasks)
        phi = None
        if u < UNITS:
            pq, phi = project(wq_s, u % GROUPS, u // GROUPS, first), []
            last += [(QUERY_SLOTS[j] - NOPS, task(features, pq[j], phi)) for j in range(4)]
        else:
            for _, fn in first:
                fn()
        if u >= GROUPS:
            i, cols = divmod(u - GROUPS, GROUPS)
            attn = block_product(task(attention_operand, i), lambda n: wo_s[at(cols * NOPS + n)], last)
        else:
            for _, fn in last:
                fn()
            for k in range(4 * u, 4 * u + 4):
                modulation(2 * D + 256 * k)
            if u == GROUPS - 1:
                score_bias = output_vectors()
        if u == (EARLY_TILES + 2) * GROUPS - 1:
            cp_out[0].start()
            wait_all(cp_ffn)
    add_residual(attn, TILES - 1, GROUPS - 1)
    for fn in (mean_attended, score_rows):
        for r0 in range(S - T, S, LAST_ROWS):
            fn(r0, LAST_ROWS)

    scores = jnp.concatenate(top[0::2], axis=0)
    tokens = jnp.concatenate(top[1::2], axis=0)

    def take_top(scores):
        score = jnp.max(scores, axis=0, keepdims=True)
        token = jnp.min(jnp.where(scores == score, tokens, S - 1).astype(F32), axis=0, keepdims=True)
        return score, token.astype(I32)

    score0, token0 = take_top(scores)
    score1, token1 = take_top(jnp.where(tokens == token0, -jnp.inf, scores))
    cp_out[1].start()
    routed = [jnp.clip(token[0, 0], 0, S - 1) for token in (token0, token1)]

    row16 = _iota((16, D), 0)
    shift, scale, gate_b = mod_b[at(1)], mod_b[at(2)], mod_b[at(3)]
    x1_sel = h2_sel = weight = jnp.zeros((16, D), F32)
    for k, (t, score) in enumerate(zip(routed, (score0, score1))):
        blk, row = t // (2 * T) * 16 + t % T // 16, pl.ds(t % 16, 1)
        x1 = jnp.where(t // T % 2 == 0, x1_v[0][blk, row, :], x1_v[1][blk, row, :])
        mean, inv = (jnp.tile(stat_v[m, t // 8, pl.ds(t % 8, 1), :], (1, D // 128)) for m in range(2))
        x1_sel = jnp.where(row16 == k, x1, x1_sel)
        h2_sel = jnp.where(row16 == k, (x1 - mean) * inv * scale[:1] + shift[:1], h2_sel)
        weight = jnp.where(row16 == k, jnp.tile(jax.nn.sigmoid(score), (1, D // 128)), weight)
    h_sel = h2_sel.astype(BF16)
    gate_b = jnp.concatenate([gate_b, gate_b], axis=0)
    base_rows, update_scale = x1_sel + gate_b * h2_sel, gate_b * weight

    def down(f, act):
        return _dot(act, wd_v[f * F_CHUNK:(f + 1) * F_CHUNK, :], _NN)

    y, act = jnp.zeros((16, D), F32), None
    for f in range(F // F_CHUNK):
        gate, up = (_dot(h_sel, w[:, f * F_CHUNK:(f + 1) * F_CHUNK], _NN) for w in (wg_v, wu_v))
        if f > 0:
            y = y + down(f - 1, act)
        act = (gate * jax.nn.sigmoid(gate) * up).astype(BF16)
        if f < T // LAST_ROWS:
            output_rows(S - T + f * LAST_ROWS, LAST_ROWS, gate[:8, :1])
        if f == T // LAST_ROWS:
            cp_out[2].start()
    routed_rows = base_rows + update_scale * (y + down(F // F_CHUNK - 1, act))

    wait_all(cp_out)
    for k, t in enumerate(routed):
        row = jnp.broadcast_to(routed_rows[k:k + 1], (16, D))
        out_v[t // 16] = jnp.where(row16 == t % 16, row, out_v[t // 16].astype(F32)).astype(BF16)
    fix = [copy(out_v.at[t // 16], out_hbm.at[t // 16]) for t in routed]
    fix[0].start()

    @pl.when(routed[0] // 16 != routed[1] // 16)
    def _():
        fix[1].start()
        fix[1].wait()

    fix[0].wait()


@jax.jit
def pallas_adaLN_cond__linear_kernel_hedgehog__moe_arch_mod__prompt_kernel(
    A_x: jax.Array,
    A_wqkv: jax.Array,
    A_w_phi: jax.Array,
    A_wo: jax.Array,
    B_x: jax.Array,
    B_w_r: jax.Array,
    B_w_gate: jax.Array,
    B_w_up: jax.Array,
    B_w_down: jax.Array,
    c: jax.Array,
    w_mod: jax.Array,
):
    del B_x
    weight_operands = pltpu.VMEM((GROUPS * NOPS, 64, HALF), U32)
    out = pl.pallas_call(
        _kernel,
        out_shape=jax.ShapeDtypeStruct((S // 16, 16, D), BF16),
        in_specs=[pl.BlockSpec(memory_space=pl.ANY)] * 10,
        out_specs=pl.BlockSpec(memory_space=pl.ANY),
        scratch_shapes=[
            pltpu.VMEM((S // 16 + 1, 16, D), BF16),
            pltpu.VMEM((3 * D // 128 + 1, D, 128), BF16),
            pltpu.VMEM((H * DH, DH), BF16),
            pltpu.VMEM((GROUPS + 1, 256, D), BF16),
            pltpu.VMEM((D // 128, 128), BF16),
            pltpu.VMEM((D, F), BF16),
            pltpu.VMEM((D, F), BF16),
            pltpu.VMEM((F, D), BF16),
            pltpu.VMEM((1, D), BF16),
            pltpu.VMEM((6 * D // 128, D, 128), BF16),
            weight_operands,
            weight_operands,
            weight_operands,
            weight_operands,
            pltpu.VMEM((S // 16, 16, D), BF16),
            pltpu.VMEM((2, 8, D), F32),
            pltpu.VMEM((7, 8, D), F32),
            pltpu.VMEM((H // 2, 40, 128), U32),
            pltpu.VMEM((2, S // 8, 8, 128), F32),
            pltpu.SemaphoreType.DMA((40,)),
            *[pltpu.VMEM((S // 32 + 1, 16, D), F32)] * 2,
            *[pltpu.VMEM((GROUPS, 80, 128), F32)] * 4,
            *[pltpu.VMEM((NOPS, 64, HALF), U32)] * TILES,
        ],
        compiler_params=pltpu.CompilerParams(vmem_limit_bytes=120 * 1024 * 1024),
        name="hedgehog_moe",
    )(
        A_x.reshape(S // 16, 16, D), A_wqkv, A_w_phi.reshape(H * DH, DH),
        A_wo.reshape(GROUPS, 256, D), B_w_r.reshape(D // 128, 128),
        B_w_gate, B_w_up, B_w_down, c, w_mod,
    )
    return out.reshape(1, S, D)
```

```python
import functools
import itertools
import math

import jax
import jax.numpy as jnp
from jax import lax
import jax.experimental.pallas as pl
import jax.experimental.pallas.tpu as pltpu

S, D, H, DH, F = 2048, 1024, 32, 32, 3584
T = 256
TILES = S // T
GROUPS = 4
UNITS = TILES * GROUPS
HALF = D // 2
NOPS = 7
F_CHUNK = 512
LOG2E = math.log2(math.e)

KEY_SLOTS = (9, 10, 11, 12)
NORM_SLOTS = (1,)
NORM_SLOTS_EARLY = (2, 11)
NORM_SLOTS_LATE = (13, 3)
NORM_RELEASE = 5
NORM_PACE = 12
QUERY_SLOTS = (9, 10, 11, 12)
TRANSPOSE_SLOT = 6
FINISH_SLOTS = ((2, 5), (7, 13))
FINISH_RELEASE = 5
LATE_UNIT = UNITS - 12 if UNITS > 20 else UNITS - 8
EARLY_TILES = max(TILES - 3, 1)
LAST_ROWS = 64

F32 = jnp.float32
BF16 = jnp.bfloat16
U32 = jnp.uint32
I32 = jnp.int32

_NN = (((1,), (0,)), ((), ()))
_NT = (((1,), (1,)), ((), ()))


def _dot(a, b, dims):
    return lax.dot_general(a, b, dims, preferred_element_type=F32)


def _round_bf16(x):
    return x.astype(BF16).astype(F32)


def _bits(x):
    return pltpu.bitcast(x, U32)


def _bf16(words):
    return pltpu.bitcast(words, BF16)


def _iota(shape, axis):
    return lax.broadcasted_iota(I32, shape, axis)


def _recip(x):
    return pl.reciprocal(x, full_range=False)


def _join(tokens):
    return functools.reduce(jnp.bitwise_or, tokens)


def _left_operands(a11, a12, a21, a22):
    return a11 + a22, a21 + a22, a11, a22, a11 + a12, a21 - a11, a12 - a22


def _right_operands(b11, b12, b21, b22):
    return b11 + b22, b11, b12 - b22, b21 - b11, b22, b11 + b12, b21 + b22


def _row_sum(x):
    return jnp.sum(x, axis=-1, keepdims=True)


def _inv_std(centered):
    return lax.rsqrt(_row_sum(centered * centered) * (1.0 / D) + 1e-5)


def _head_allreduce(x, op):
    r = functools.reduce(op, [x[i:i + 8] for i in range(0, 64, 8)])
    r = op(r, pltpu.roll(r, 4, 0))
    return op(r, pltpu.roll(r, 2, 0))


def _feature_map(p):
    p3 = p.reshape(8, 8, T)
    e_pos = jnp.exp2(p3 - _head_allreduce(p, jnp.maximum)[None])
    e_neg = jnp.exp2(_head_allreduce(p, jnp.minimum)[None] - p3)
    inv_pos, inv_neg = (_recip(_head_allreduce(e.reshape(64, T), jnp.add)) for e in (e_pos, e_neg))
    phi = jnp.concatenate([e_pos * inv_pos[None], e_neg * inv_neg[None]], axis=0)
    token = _bits(inv_pos) | _bits(inv_neg)
    return phi.reshape(2 * 64, T).astype(BF16), token[:, :128] | token[:, 128:]


def _kernel(x_hbm, wqkv_hbm, wphi_hbm, wo_hbm, wr_hbm, wg_hbm, wu_hbm, wd_hbm, c_hbm, wmod_hbm,
            out_hbm,
            x_v, wqkv_v, wphi_v, wo_v, wr_v, wg_v, wu_v, wd_v, c_v, wmod_v,
            wq_s, wk_s, wv_s, wo_s, out_v, mod_a, mod_b, kv_s, stat_v,
            sems, *rest):
    x1_v, kv_acc, h_s = rest[:2], rest[2:6], rest[6:]
    task = functools.partial

    sem_ids = itertools.count()

    def copy(src, dst):
        return pltpu.make_async_copy(src, dst, sems.at[next(sem_ids)])

    def copy_blocks(src, dst, start, stop):
        return copy(src.at[pl.ds(start, stop - start)], dst.at[pl.ds(start, stop - start)])

    def copy_slabs(src, dst, first, count):
        sem = sems.at[next(sem_ids)]
        return [pltpu.make_async_copy(src.at[:, pl.ds(k * 128, 128)], dst.at[k], sem)
                for k in range(first, first + count)]

    def wait_all(copies):
        for cp in copies:
            cp.wait()

    mod_a_cols = [c0 + l for l in (0, 256) for c0 in range(0, 2 * D, HALF)]
    cp_c, cp_phi, cp_wr = copy(c_hbm, c_v), copy(wphi_hbm, wphi_v), copy(wr_hbm, wr_v)
    cp_x = [copy_blocks(x_hbm, x_v, *span) for span in ((0, 16), (16, 32), (32, S // 16))]
    cp_mod_a = [copy_slabs(wmod_hbm, wmod_v, c0 // 128, 2) for c0 in mod_a_cols]
    cp_wk = [copy_slabs(wqkv_hbm, wqkv_v, 8 + 2 * g, 2) for g in range(GROUPS)]
    cp_wv = [copy_slabs(wqkv_hbm, wqkv_v, 16 + 2 * g, 2) for g in range(GROUPS)]
    cp_late = (copy_slabs(wqkv_hbm, wqkv_v, 0, 8) + copy_slabs(wmod_hbm, wmod_v, 16, 32)
               + [cp_wr, copy_blocks(wo_hbm, wo_v, 0, GROUPS)])
    cp_ffn = [copy(wg_hbm, wg_v), copy(wu_hbm, wu_v), copy(wd_hbm, wd_v)]
    cp_out = [copy_blocks(out_v, out_hbm, 16 * first, 16 * stop) for first, stop in
              ((0, EARLY_TILES), (EARLY_TILES, TILES - 1), (TILES - 1, TILES))]
    for cp in (cp_c, cp_x[0], cp_phi, *itertools.chain(*cp_mod_a[:4]), *cp_wk[0],
               *itertools.chain(*cp_mod_a[4:]), *cp_wv[0], *cp_wk[1], *cp_wv[1], cp_x[1],
               *cp_wk[2], *cp_wv[2], *cp_wk[3], *cp_wv[3], cp_x[2], *cp_late, *cp_ffn):
        cp.start()

    cp_c.wait()
    c = c_v[...].astype(F32)
    silu_c = jnp.broadcast_to(c * jax.nn.sigmoid(c), (16, D)).astype(BF16)

    never = jnp.broadcast_to(c[:, :128] * c[:, :128], (8, 128)) < 0.0
    zero = jnp.max(never.astype(F32)).astype(I32)
    stamps = itertools.count(1)
    history, due = [], {}

    def at(i):
        return i + zero * next(stamps)

    def after(words, token):
        head = jnp.concatenate([jnp.where(never, token, words[:8, l:l + 128])
                                for l in range(0, words.shape[1], 128)], axis=1)
        return jnp.concatenate([head, words[8:]], axis=0)

    def hold(ref, token):
        token = pltpu.bitcast(token, ref.dtype)
        ref[ref.shape[0] - 1, :token.shape[0], :128] = token

    def once(stat, token):
        return jnp.where(never[:, :1], token, stat)

    def tick(back, step=0):
        back, step = back - step // 16, step % 16
        return history[-back][8 * step:8 * step + 8, :128]

    def block_product(left, right, tasks):
        assert all(0 <= entry[0] < NOPS for entry in tasks)

        def m(n, slot):
            for at_slot, fn, *slack in tasks:
                if at_slot == slot:
                    due.setdefault(len(history) + sum(slack), []).append(fn())
            tokens = [t for t in due.pop(len(history), []) if t is not None]
            operands = [left(n), right(n)]
            for k, op in enumerate(operands):
                if op.dtype == U32:
                    operands[k] = _bf16(after(op, _join(tokens)) if tokens else op)
                    tokens = []
            history.append(_dot(*operands, _NT))
            return history[-1]

        m2, m4 = m(1, 0), m(3, 1)
        c21 = m2 + m4
        m3 = m(2, 2)
        c22 = m3 - m2
        m5 = m(4, 3)
        c12 = m3 + m5
        c11 = m4 - m5
        m1 = m(0, 4)
        c11, c22 = c11 + m1, c22 + m1
        c11 = c11 + m(6, 5)
        c22 = c22 + m(5, 6)
        return c11, c12, c21, c22

    def split_tasks(tasks):
        return ([t for t in tasks if t[0] < NOPS],
                [(t[0] - NOPS, *t[1:]) for t in tasks if t[0] >= NOPS])

    def modulation(col0):
        i, c0 = divmod(col0, D)
        w = jnp.concatenate([wmod_v[at(col0 // 128 + k)] for k in range(2)], axis=1)
        m = _round_bf16(_dot(silu_c, w, _NN)[:8])
        dst, row = (mod_a, i) if i < 2 else (mod_b, i - 2)
        dst[row, :, c0:c0 + 256] = _round_bf16(1.0 + m) if i % 3 == 1 else m

    def phi_blocks():
        select = (_iota((128, DH), 0) % 64 // 2 == _iota((128, DH), 1)).astype(BF16)
        row = _iota((128, 128), 0)
        same_head = row // 64 * 2 + row % 2 == _iota((128, 128), 1) // DH
        return [jnp.where(same_head, _dot(select, wphi_v[k * 128:(k + 1) * 128, :], _NT), 0.0)
                .astype(BF16) for k in range(D // 128)]

    def fold_phi(col0, dst, g, l):
        quads = []
        for k in (2 * g, 2 * g + 1):
            w = jnp.concatenate([wqkv_v[at(col0 // 128 + k), r:r + 128, :]
                                 for r in (l * 128, HALF + l * 128)], axis=0)
            folded = _dot(phi_bd[k], w, _NT) * LOG2E
            quads += [folded[:, :128], folded[:, 128:]]
        for n, op in enumerate(_left_operands(*quads)):
            dst[g * NOPS + n, :, l * 128:(l + 1) * 128] = _bits(op.astype(BF16))

    def transpose_wv(g):
        first, second = (wqkv_v[at(16 + 2 * g + k)].astype(F32) for k in range(2))
        ops = _left_operands(first[:HALF], first[HALF:], second[:HALF], second[HALF:])
        for n, op in enumerate(ops):
            wv_s[g * NOPS + n] = _bits(op.astype(BF16).T)

    def transpose_wo(cols, g):
        hold(wo_v, tick(1))
        w = wo_v[at(g), :, cols * 256:(cols + 1) * 256].astype(F32)
        ops = _right_operands(w[:128, :128], w[:128, 128:], w[128:, :128], w[128:, 128:])
        for n, op in enumerate(ops):
            wo_s[cols * NOPS + n, :, g * 128:(g + 1) * 128] = _bits(op.astype(BF16).T)

    stats = {}

    def load_rows(i, b, n):
        return jnp.concatenate([x_v[pl.ds(at(i * 16 + half * 8 + b), n)].astype(F32)
                                for half in range(2)], axis=0).reshape(4 * n, 8, D)

    def row_statistics(i, b, n):
        mean = _row_sum(load_rows(i, b, n)) * (1.0 / D)
        stats[i, b] = mean, _inv_std(load_rows(i, b, n) - mean)

    def normalize_rows(i, b, n, column_groups, back=0):
        mean, inv = stats[i, b]
        mean = once(mean, inv)
        x = load_rows(i, b, n)
        for l in column_groups:
            m = once(mean, tick(back, NORM_PACE * l)[None, :, :1]) if back else mean
            lo, hi = (((x[:, :, c0:c0 + 256] - m) * inv * mod_a[at(1), :, c0:c0 + 256][None]
                       + mod_a[at(0), :, c0:c0 + 256][None]).reshape(32 * n, 256)
                      for c0 in (l * 256, HALF + l * 256))
            ops = _right_operands(lo[:16 * n], lo[16 * n:], hi[:16 * n], hi[16 * n:])
            for k, op in enumerate(ops):
                h_s[i][k, 8 * b:8 * (b + n), l * 256:(l + 1) * 256] = _bits(op.astype(BF16))

    def layer_norm_rows(i, b, n):
        hold(x_v, tick(NORM_RELEASE))
        row_statistics(i, b, n)
        normalize_rows(i, b, n, (0, 1), back=2)
        return h_s[i][at(0), 8 * b:8 * (b + 1), :128]

    def project(w_s, g, i, tasks):
        blocks = block_product(lambda n: w_s[at(g * NOPS + n)], lambda n: h_s[i][at(n)], tasks)
        return [jnp.concatenate([blocks[j // 2 * 2 + half][j % 2 * 64:(j % 2 + 1) * 64]
                                 for half in range(2)], axis=1) for j in range(4)]

    def features(p, out):
        phi, token = _feature_map(p)
        out.append(phi)
        return token

    def accumulate_kv(v, phi, g, i):
        for j in range(4):
            values = jnp.concatenate([v[j], jnp.ones((16, T), F32)], axis=0).astype(BF16)
            kv = _dot(values, phi[j], _NT)
            kv = kv if i == 0 else kv_acc[j][at(g)] + kv
            if i + 1 < TILES:
                kv_acc[j][g] = kv
            else:
                row = _iota((80, 128), 0)
                head = jnp.where(row < 64, row // DH, row // 8 % 2)
                kv_s[4 * g + j] = _bits(
                    jnp.where(head == _iota((80, 128), 1) % 2, kv, 0.0).astype(BF16))

    cp_x[0].wait()
    for b in range(0, 8, 2):
        row_statistics(0, b, 2)
    cp_phi.wait()
    phi_bd = phi_blocks()
    for l in range(2):
        for k in range(4 * l, 4 * l + 4):
            wait_all(cp_mod_a[k])
            modulation(mod_a_cols[k])
        for b in range(0, 8, 2):
            normalize_rows(0, b, 2, (l,))
        if l == 0:
            wait_all(cp_wk[0])
            for k in range(HALF // 128):
                fold_phi(D, wk_s, 0, k)
    wait_all(cp_wv[0])

    pending = None
    for u in range(UNITS):
        i, g = divmod(u, GROUPS)
        if 0 < u < GROUPS:
            wait_all(cp_wk[g] + cp_wv[g] + cp_x[1:2] * (g == 2))
            for l in range(HALF // 128):
                fold_phi(D, wk_s, g, l)
        if u == GROUPS + 2:
            cp_x[2].wait()
        if u == LATE_UNIT:
            wait_all(cp_late)
        if LATE_UNIT <= u < LATE_UNIT + 8:
            hold(wqkv_v, tick(13))
            for k in range(2 * (u - LATE_UNIT), 2 * (u - LATE_UNIT + 1)):
                fold_phi(0, wq_s, *divmod(k, HALF // 128))

        if i < 2:
            work = zip(NORM_SLOTS_EARLY, (4 * g - 8, 4 * g - 6), (2, 2), (3, 3)) if g >= 2 else ()
        elif i + 1 < TILES:
            slots = NORM_SLOTS_LATE if u >= LATE_UNIT else NORM_SLOTS
            n = 2 // len(slots)
            work = [(slot, 2 * g + k, n, 2 + n) for k, slot in enumerate(slots)]
        else:
            work = ()
        first, last = split_tasks([(slot, task(layer_norm_rows, i + 1, b, n), slack)
                                   for slot, b, n, slack in work])
        pk = project(wk_s, g, i, first)
        if i == 0:
            transpose_wv(g)
        if pending is not None:
            accumulate_kv(*pending)
        phi = []
        last += [(KEY_SLOTS[j] - NOPS, task(features, pk[j], phi)) for j in range(4)]
        if i == TILES - 1:
            last += [(3 + k, task(transpose_wo, g, k)) for k in range(GROUPS)]
        pending = project(wv_s, g, i, last), phi, g, i
    accumulate_kv(*pending)

    o_parts, o_ops = {}, {}
    top = [jnp.full((8, 128), -jnp.inf, F32), jnp.zeros((8, 128), I32)] * 2

    def output_vectors():
        wr = wr_v[...].astype(F32)
        wr = jnp.concatenate([jnp.broadcast_to(wr[l:l + 1], (8, 128)) for l in range(D // 128)], axis=1)
        shift, scale, gate = mod_b[1], mod_b[2], mod_b[3]
        mod_b[4] = scale * wr
        mod_b[5] = scale * gate
        mod_b[6] = shift * gate
        return _row_sum(shift * wr), _row_sum(scale * wr)

    def attend(phi, g, out):
        out.extend(_dot(_bf16(kv_s[at(4 * g + j)]), phi[j], _NN) for j in range(4))

    def transpose_attention(nums, i, g):
        blocks = []
        for num in nums:
            num = num.reshape(10, 8, T)
            inv = _recip(num[8:] + 1e-6)
            o = jnp.concatenate([num[:4] * inv[0:1], num[4:8] * inv[1:2]], axis=0)
            blocks.append(o.reshape(64, T))
        first = jnp.concatenate(blocks[:2], axis=0).T
        second = jnp.concatenate(blocks[2:], axis=0).T
        quads = first[:128], second[:128], first[128:], second[128:]
        o_parts[i, g] = _left_operands(*quads)
        return _join([_bits(q[120:]) for q in quads])

    def attention_operand(i, n):
        if (i, n) not in o_ops:
            parts = [o_parts[i, g][n] for g in range(GROUPS)]
            o_ops[i, n] = jnp.concatenate(parts, axis=1).astype(BF16)
        return o_ops[i, n]

    def add_residual(blocks, i, cols):
        for k in (2, 1, 0, 3):
            hold(x_v, blocks[k][:8])
            cs = pl.ds(cols * 256 + k % 2 * 128, 128)
            x = x_v[pl.ds(at(i * 16 + k // 2 * 8), 8), :, cs].astype(F32).reshape(16, 8, 128)
            x1 = x + mod_b[at(0), :, cs][None] * blocks[k].reshape(16, 8, 128)
            x1_v[i % 2][pl.ds(i // 2 * 16 + k // 2 * 8, 8), :, cs] = x1.reshape(8, 16, 128)
            if i == TILES - 1:
                accumulate_moments(k // 2, x1, cs)

    moments = {}

    def accumulate_moments(half, x1, cs):
        if half not in moments:
            moments[half] = [_row_sum(x1) * (1.0 / 128), None]
        pivot, sums = moments[half]
        d = x1 - pivot
        terms = d, d * d, d * mod_b[at(4), :, cs][None]
        moments[half][1] = terms if sums is None else [s + t for s, t in zip(sums, terms)]

    def load_attended(r0, n):
        i = r0 // T
        return x1_v[i % 2][pl.ds(at(i // 2 * 16 + r0 % T // 16), n // 16)].reshape(n // 8, 8, D)

    def mean_attended(r0, n):
        hold(x1_v[r0 // T % 2], tick(FINISH_RELEASE))
        stats[r0] = _row_sum(load_attended(r0, n)) * (1.0 / D)
        return _join([_bits(jnp.broadcast_to(stats[r0][k], (8, 128))) for k in range(n // 8)])

    def score_rows(r0, n):
        if r0 < S - T:
            mean = stats[r0]
            centered = load_attended(r0, n) - mean
            routed = _row_sum(centered * mod_b[at(4)][None])
            inv = _inv_std(centered)
        else:
            pivot, sums = moments[r0 % T // 128]
            rows = slice(r0 % 128 // 8, (r0 % 128 + n) // 8)
            offset, square, routed = (_row_sum(s[rows]) for s in sums)
            offset = offset * (1.0 / D)
            mean = pivot[rows] + offset
            inv = lax.rsqrt(jnp.maximum(square * (1.0 / D) - offset * offset, 0.0) + 1e-5)
            routed = routed - offset * route_sum
        for k, stat in enumerate((mean, inv)):
            stat_v[k, pl.ds(r0 // 8, n // 8)] = jnp.broadcast_to(stat, (n // 8, 8, 128))
        stats[r0] = mean, inv
        score = _round_bf16(routed * inv + score_bias)
        best, best_i, second, second_i = top
        for b in range(n // 8):
            s, t = jnp.broadcast_to(score[b], (8, 128)), _iota((8, 128), 0) + (r0 + 8 * b)
            above_best, above_second = s > best, s > second
            second = jnp.where(above_best, best, jnp.where(above_second, s, second))
            second_i = jnp.where(above_best, best_i, jnp.where(above_second, t, second_i))
            best = jnp.where(above_best, s, best)
            best_i = jnp.where(above_best, t, best_i)
        top[:] = best, best_i, second, second_i

    def output_rows(r0, n, token=None):
        mean, inv = stats[r0]
        if token is not None:
            inv = once(inv, token[None])
        x1 = load_attended(r0, n)
        out = x1 + ((x1 - once(mean, inv)) * inv * mod_b[at(5)][None] + mod_b[at(6)][None])
        out_v[pl.ds(r0 // 16, n // 16)] = out.reshape(n // 16, 16, D).astype(BF16)

    def finish_rows(r0, n):
        score_rows(r0, n)
        output_rows(r0, n)
        return _bits(top[3]) | _bits(out_v[at(0), :, :128])

    phi = attn = None
    for u in range(UNITS + GROUPS):
        tasks = []
        if phi is not None:
            nums = []
            tasks += [(0, task(attend, phi, (u - 1) % GROUPS, nums)),
                      (TRANSPOSE_SLOT, task(transpose_attention, nums, *divmod(u - 1, GROUPS)))]
        if attn is not None:
            add_residual(attn, *divmod(u - GROUPS - 1, GROUPS))
        if u >= 2 * GROUPS:
            n = 64 // len(FINISH_SLOTS)
            for k, slots in enumerate(FINISH_SLOTS):
                for slot, fn in zip(slots, (mean_attended, finish_rows)):
                    tasks.append((slot if u < UNITS else NOPS + slot // 2,
                                  task(fn, (u - 2 * GROUPS) * 64 + n * k, n)))
        first, last = split_tasks(tasks)
        phi = None
        if u < UNITS:
            pq, phi = project(wq_s, u % GROUPS, u // GROUPS, first), []
            last += [(QUERY_SLOTS[j] - NOPS, task(features, pq[j], phi)) for j in range(4)]
        else:
            for _, fn in first:
                fn()
        if u >= GROUPS:
            i, cols = divmod(u - GROUPS, GROUPS)
            attn = block_product(task(attention_operand, i), lambda n: wo_s[at(cols * NOPS + n)], last)
        else:
            for _, fn in last:
                fn()
            for k in range(4 * u, 4 * u + 4):
                modulation(2 * D + 256 * k)
            if u == GROUPS - 1:
                score_bias, route_sum = output_vectors()
        if u == (EARLY_TILES + 2) * GROUPS - 1:
            cp_out[0].start()
            wait_all(cp_ffn)
    add_residual(attn, TILES - 1, GROUPS - 1)
    for r0 in range(S - T, S, LAST_ROWS):
        score_rows(r0, LAST_ROWS)

    scores = jnp.concatenate(top[0::2], axis=0)
    tokens = jnp.concatenate(top[1::2], axis=0)

    def take_top(scores):
        score = jnp.max(scores, axis=0, keepdims=True)
        token = jnp.min(jnp.where(scores == score, tokens, S - 1).astype(F32), axis=0, keepdims=True)
        return score, token.astype(I32)

    score0, token0 = take_top(scores)
    score1, token1 = take_top(jnp.where(tokens == token0, -jnp.inf, scores))
    cp_out[1].start()
    routed = [jnp.clip(token[0, 0], 0, S - 1) for token in (token0, token1)]

    row16 = _iota((16, D), 0)
    shift, scale, gate_b = mod_b[at(1)], mod_b[at(2)], mod_b[at(3)]
    x1_sel = h2_sel = weight = jnp.zeros((16, D), F32)
    for k, (t, score) in enumerate(zip(routed, (score0, score1))):
        blk, row = t // (2 * T) * 16 + t % T // 16, pl.ds(t % 16, 1)
        x1 = jnp.where(t // T % 2 == 0, x1_v[0][blk, row, :], x1_v[1][blk, row, :])
        mean, inv = (jnp.tile(stat_v[m, t // 8, pl.ds(t % 8, 1), :], (1, D // 128)) for m in range(2))
        x1_sel = jnp.where(row16 == k, x1, x1_sel)
        h2_sel = jnp.where(row16 == k, (x1 - mean) * inv * scale[:1] + shift[:1], h2_sel)
        weight = jnp.where(row16 == k, jnp.tile(jax.nn.sigmoid(score), (1, D // 128)), weight)
    h_sel = h2_sel.astype(BF16)
    gate_b = jnp.concatenate([gate_b, gate_b], axis=0)
    base_rows, update_scale = x1_sel + gate_b * h2_sel, gate_b * weight

    def down(f, act):
        return _dot(act, wd_v[f * F_CHUNK:(f + 1) * F_CHUNK, :], _NN)

    y, act = jnp.zeros((16, D), F32), None
    for f in range(F // F_CHUNK):
        gate, up = (_dot(h_sel, w[:, f * F_CHUNK:(f + 1) * F_CHUNK], _NN) for w in (wg_v, wu_v))
        if f > 0:
            y = y + down(f - 1, act)
        act = (gate * jax.nn.sigmoid(gate) * up).astype(BF16)
        if f < T // LAST_ROWS:
            output_rows(S - T + f * LAST_ROWS, LAST_ROWS, gate[:8, :1])
        if f == T // LAST_ROWS:
            cp_out[2].start()
    routed_rows = base_rows + update_scale * (y + down(F // F_CHUNK - 1, act))

    wait_all(cp_out)
    for k, t in enumerate(routed):
        row = jnp.broadcast_to(routed_rows[k:k + 1], (16, D))
        out_v[t // 16] = jnp.where(row16 == t % 16, row, out_v[t // 16].astype(F32)).astype(BF16)
    fix = [copy(out_v.at[t // 16], out_hbm.at[t // 16]) for t in routed]
    fix[0].start()

    @pl.when(routed[0] // 16 != routed[1] // 16)
    def _():
        fix[1].start()
        fix[1].wait()

    fix[0].wait()


@jax.jit
def pallas_adaLN_cond__linear_kernel_hedgehog__moe_arch_mod__prompt_kernel(
    A_x: jax.Array,
    A_wqkv: jax.Array,
    A_w_phi: jax.Array,
    A_wo: jax.Array,
    B_x: jax.Array,
    B_w_r: jax.Array,
    B_w_gate: jax.Array,
    B_w_up: jax.Array,
    B_w_down: jax.Array,
    c: jax.Array,
    w_mod: jax.Array,
):
    del B_x
    weight_operands = pltpu.VMEM((GROUPS * NOPS, 64, HALF), U32)
    out = pl.pallas_call(
        _kernel,
        out_shape=jax.ShapeDtypeStruct((S // 16, 16, D), BF16),
        in_specs=[pl.BlockSpec(memory_space=pl.ANY)] * 10,
        out_specs=pl.BlockSpec(memory_space=pl.ANY),
        scratch_shapes=[
            pltpu.VMEM((S // 16 + 1, 16, D), BF16),
            pltpu.VMEM((3 * D // 128 + 1, D, 128), BF16),
            pltpu.VMEM((H * DH, DH), BF16),
            pltpu.VMEM((GROUPS + 1, 256, D), BF16),
            pltpu.VMEM((D // 128, 128), BF16),
            pltpu.VMEM((D, F), BF16),
            pltpu.VMEM((D, F), BF16),
            pltpu.VMEM((F, D), BF16),
            pltpu.VMEM((1, D), BF16),
            pltpu.VMEM((6 * D // 128, D, 128), BF16),
            weight_operands,
            weight_operands,
            weight_operands,
            weight_operands,
            pltpu.VMEM((S // 16, 16, D), BF16),
            pltpu.VMEM((2, 8, D), F32),
            pltpu.VMEM((7, 8, D), F32),
            pltpu.VMEM((H // 2, 40, 128), U32),
            pltpu.VMEM((2, S // 8, 8, 128), F32),
            pltpu.SemaphoreType.DMA((40,)),
            *[pltpu.VMEM((S // 32 + 1, 16, D), F32)] * 2,
            *[pltpu.VMEM((GROUPS, 80, 128), F32)] * 4,
            *[pltpu.VMEM((NOPS, 64, HALF), U32)] * TILES,
        ],
        compiler_params=pltpu.CompilerParams(vmem_limit_bytes=120 * 1024 * 1024),
        name="hedgehog_moe",
    )(
        A_x.reshape(S // 16, 16, D), A_wqkv, A_w_phi.reshape(H * DH, DH),
        A_wo.reshape(GROUPS, 256, D), B_w_r.reshape(D // 128, 128),
        B_w_gate, B_w_up, B_w_down, c, w_mod,
    )
    return out.reshape(1, S, D)
```

```python
import functools
import itertools
import math

import jax
import jax.numpy as jnp
from jax import lax
import jax.experimental.pallas as pl
import jax.experimental.pallas.tpu as pltpu

S, D, H, DH, F = 2048, 1024, 32, 32, 3584
T = 256
TILES = S // T
GROUPS = 4
UNITS = TILES * GROUPS
HALF = D // 2
NOPS = 7
F_CHUNK = 512
LOG2E = math.log2(math.e)

KEY_SLOTS = (9, 10, 11, 12)
NORM_SLOTS = (1,)
NORM_SLOTS_EARLY = (2, 11)
NORM_SLOTS_LATE = (13, 3)
NORM_RELEASE = 5
NORM_PACE = 12
QUERY_SLOTS = (9, 10, 12, 13)
ATTEND_SLOTS = (0, 6)
ATTEND_SLOTS_LAST = (7, 11)
FINISH_SLOTS = ((2, 5), (7, 13))
FINISH_SLOTS_LAST = ((9, 10), (11, 13))
FINISH_ROWS_LAST = (32, 48, 48, 0)
FINISH_RELEASE = 5
KEY_WEIGHT_SLOT, X_WAIT_SLOT, LATE_WAIT_SLOT, OUTPUT_SLOT = 12, 3, 6, 4
LATE_UNIT = UNITS - 12
LAG = 6
EARLY_TILES = TILES - 3
LAST_ROWS = 64

F32 = jnp.float32
BF16 = jnp.bfloat16
U32 = jnp.uint32
I32 = jnp.int32

_NN = (((1,), (0,)), ((), ()))
_NT = (((1,), (1,)), ((), ()))


def _dot(a, b, dims):
    return lax.dot_general(a, b, dims, preferred_element_type=F32)


def _round_bf16(x):
    return x.astype(BF16).astype(F32)


def _bits(x):
    return pltpu.bitcast(x, U32)


def _bf16(words):
    return pltpu.bitcast(words, BF16)


def _iota(shape, axis):
    return lax.broadcasted_iota(I32, shape, axis)


def _recip(x):
    return pl.reciprocal(x, full_range=False)


def _join(tokens):
    return functools.reduce(jnp.bitwise_or, tokens)


def _left_operands(a11, a12, a21, a22):
    return a11 + a22, a21 + a22, a11, a22, a11 + a12, a21 - a11, a12 - a22


def _right_operands(b11, b12, b21, b22):
    return b11 + b22, b11, b12 - b22, b21 - b11, b22, b11 + b12, b21 + b22


def _row_sum(x):
    return jnp.sum(x, axis=-1, keepdims=True)


def _inv_std(centered):
    return lax.rsqrt(_row_sum(centered * centered) * (1.0 / D) + 1e-5)


def _head_allreduce(x, op):
    r = functools.reduce(op, [x[i:i + 8] for i in range(0, 64, 8)])
    r = op(r, pltpu.roll(r, 4, 0))
    return op(r, pltpu.roll(r, 2, 0))


def _feature_map(p):
    p3 = p.reshape(8, 8, T)
    e_pos = jnp.exp2(p3 - _head_allreduce(p, jnp.maximum)[None])
    e_neg = jnp.exp2(_head_allreduce(p, jnp.minimum)[None] - p3)
    inv_pos, inv_neg = (_recip(_head_allreduce(e.reshape(64, T), jnp.add)) for e in (e_pos, e_neg))
    phi = jnp.concatenate([e_pos * inv_pos[None], e_neg * inv_neg[None]], axis=0)
    token = _bits(inv_pos) | _bits(inv_neg)
    return phi.reshape(2 * 64, T).astype(BF16), token[:, :128] | token[:, 128:]


def _kernel(x_hbm, wqkv_hbm, wphi_hbm, wo_hbm, wr_hbm, wg_hbm, wu_hbm, wd_hbm, c_hbm, wmod_hbm,
            out_hbm,
            x_v, wqkv_v, wphi_v, wo_v, wr_v, wg_v, wu_v, wd_v, c_v, wmod_v,
            wq_s, wk_s, wv_s, wo_s, out_v, mod_a, mod_b, kv_s, stat_v,
            sems, *rest):
    x1_v, kv_acc, h_s = rest[:2], rest[2:6], rest[6:]
    task = functools.partial

    sem_ids = itertools.count()

    def copy(src, dst):
        return pltpu.make_async_copy(src, dst, sems.at[next(sem_ids)])

    def copy_blocks(src, dst, start, stop):
        return copy(src.at[pl.ds(start, stop - start)], dst.at[pl.ds(start, stop - start)])

    def copy_slabs(src, dst, first, count):
        sem = sems.at[next(sem_ids)]
        return [pltpu.make_async_copy(src.at[:, pl.ds(k * 128, 128)], dst.at[k], sem)
                for k in range(first, first + count)]

    def wait_all(copies):
        for cp in copies:
            cp.wait()

    mod_a_cols = [c0 + l for l in (0, 256) for c0 in range(0, 2 * D, HALF)]
    cp_c, cp_phi, cp_wr = copy(c_hbm, c_v), copy(wphi_hbm, wphi_v), copy(wr_hbm, wr_v)
    cp_x = [[copy_blocks(x_hbm, x_v, *span) for span in spans] for spans in
            (((0, 16),), ((16, 20), (24, 28)), ((20, 24), (28, 32)), ((32, S // 16),))]
    cp_mod_a = [copy_slabs(wmod_hbm, wmod_v, c0 // 128, 2) for c0 in mod_a_cols]
    cp_wk = [copy_slabs(wqkv_hbm, wqkv_v, 8 + 2 * g, 2) for g in range(GROUPS)]
    cp_wv = [copy_slabs(wqkv_hbm, wqkv_v, 16 + 2 * g, 2) for g in range(GROUPS)]
    cp_late = (copy_slabs(wqkv_hbm, wqkv_v, 0, 8) + copy_slabs(wmod_hbm, wmod_v, 16, 32)
               + [cp_wr, copy_blocks(wo_hbm, wo_v, 0, GROUPS)])
    cp_ffn = [copy(wg_hbm, wg_v), copy(wu_hbm, wu_v), copy(wd_hbm, wd_v)]
    cp_out = [copy_blocks(out_v, out_hbm, 16 * first, 16 * stop) for first, stop in
              ((0, EARLY_TILES), (EARLY_TILES, TILES - 1), (TILES - 1, TILES))]
    for cp in (cp_c, *cp_x[0], cp_phi, *itertools.chain(*cp_mod_a[:4]), *cp_wk[0],
               *itertools.chain(*cp_mod_a[4:]), *cp_wv[0], *cp_wk[1], *cp_wv[1], *cp_x[1],
               *cp_wk[2], *cp_wv[2], *cp_x[2], *cp_wk[3], *cp_wv[3], *cp_x[3], *cp_late, *cp_ffn):
        cp.start()

    cp_c.wait()
    c = c_v[...].astype(F32)
    silu_c = jnp.broadcast_to(c * jax.nn.sigmoid(c), (16, D)).astype(BF16)

    never = jnp.broadcast_to(c[:, :128] * c[:, :128], (8, 128)) < 0.0
    zero = jnp.max(never.astype(F32)).astype(I32)
    stamps = itertools.count(1)
    history, due = [], {}

    def at(i):
        return i + zero * next(stamps)

    def after(words, token):
        head = jnp.concatenate([jnp.where(never, token, words[:8, l:l + 128])
                                for l in range(0, words.shape[1], 128)], axis=1)
        return jnp.concatenate([head, words[8:]], axis=0)

    def hold(ref, token):
        token = pltpu.bitcast(token, ref.dtype)
        ref[ref.shape[0] - 1, :token.shape[0], :128] = token

    def once(stat, token):
        return jnp.where(never[:, :1], token, stat)

    def tick(back, step=0):
        back, step = back - step // 16, step % 16
        return history[-back][8 * step:8 * step + 8, :128]

    def block_product(left, right, tasks, lower_first=False):
        assert all(0 <= entry[0] < NOPS for entry in tasks)

        def m(n, slot):
            for at_slot, fn, *slack in tasks:
                if at_slot == slot:
                    due.setdefault(len(history) + sum(slack), []).append(fn())
            tokens = [t for t in due.pop(len(history), []) if t is not None]
            operands = [left(n), right(n)]
            for k, op in enumerate(operands):
                if op.dtype == U32:
                    operands[k] = _bf16(after(op, _join(tokens)) if tokens else op)
                    tokens = []
            history.append(_dot(*operands, _NT))
            return history[-1]

        m2, m4 = m(1, 0), m(3, 1)
        c21 = m2 + m4
        m3 = m(2, 2)
        c22 = m3 - m2
        if lower_first:
            m1 = m(0, 3)
            c22 = c22 + m1 + m(5, 4)
            m5 = m(4, 5)
            return m4 + m1 - m5 + m(6, 6), m3 + m5, c21, c22
        m5 = m(4, 3)
        c12 = m3 + m5
        c11 = m4 - m5
        m1 = m(0, 4)
        c11, c22 = c11 + m1, c22 + m1
        c11 = c11 + m(6, 5)
        c22 = c22 + m(5, 6)
        return c11, c12, c21, c22

    def split_tasks(tasks):
        return ([t for t in tasks if t[0] < NOPS],
                [(t[0] - NOPS, *t[1:]) for t in tasks if t[0] >= NOPS])

    def modulation(col0):
        i, c0 = divmod(col0, D)
        w = jnp.concatenate([wmod_v[at(col0 // 128 + k)] for k in range(2)], axis=1)
        m = _round_bf16(_dot(silu_c, w, _NN)[:8])
        dst, row = (mod_a, i) if i < 2 else (mod_b, i - 2)
        dst[row, :, c0:c0 + 256] = _round_bf16(1.0 + m) if i % 3 == 1 else m

    def phi_blocks():
        select = (_iota((128, DH), 0) % 64 // 2 == _iota((128, DH), 1)).astype(BF16)
        row = _iota((128, 128), 0)
        same_head = row // 64 * 2 + row % 2 == _iota((128, 128), 1) // DH
        return [jnp.where(same_head, _dot(select, wphi_v[k * 128:(k + 1) * 128, :], _NT), 0.0)
                .astype(BF16) for k in range(D // 128)]

    def fold_phi(col0, dst, g, l):
        quads = []
        for k in (2 * g, 2 * g + 1):
            w = jnp.concatenate([wqkv_v[at(col0 // 128 + k), r:r + 128, :]
                                 for r in (l * 128, HALF + l * 128)], axis=0)
            folded = _dot(phi_bd[k], w, _NT) * LOG2E
            quads += [folded[:, :128], folded[:, 128:]]
        for n, op in enumerate(_left_operands(*quads)):
            dst[g * NOPS + n, :, l * 128:(l + 1) * 128] = _bits(op.astype(BF16))

    def transpose_wv(g):
        first, second = (wqkv_v[at(16 + 2 * g + k)].astype(F32) for k in range(2))
        ops = _left_operands(first[:HALF], first[HALF:], second[:HALF], second[HALF:])
        for n, op in enumerate(ops):
            wv_s[g * NOPS + n] = _bits(op.astype(BF16).T)

    def transpose_wo(cols, g):
        hold(wo_v, tick(1))
        w = wo_v[at(g), :, cols * 256:(cols + 1) * 256].astype(F32)
        ops = _right_operands(w[:128, :128], w[:128, 128:], w[128:, :128], w[128:, 128:])
        for n, op in enumerate(ops):
            wo_s[cols * NOPS + n, :, g * 128:(g + 1) * 128] = _bits(op.astype(BF16).T)

    stats = {}

    def load_rows(i, b, n):
        return jnp.concatenate([x_v[pl.ds(at(i * 16 + half * 8 + b), n)].astype(F32)
                                for half in range(2)], axis=0).reshape(4 * n, 8, D)

    def row_statistics(i, b, n):
        mean = _row_sum(load_rows(i, b, n)) * (1.0 / D)
        stats[i, b] = mean, _inv_std(load_rows(i, b, n) - mean)

    def normalize_rows(i, b, n, column_groups, back=0):
        mean, inv = stats[i, b]
        mean = once(mean, inv)
        x = load_rows(i, b, n)
        for l in column_groups:
            m = once(mean, tick(back, NORM_PACE * l)[None, :, :1]) if back else mean
            lo, hi = (((x[:, :, c0:c0 + 256] - m) * inv * mod_a[at(1), :, c0:c0 + 256][None]
                       + mod_a[at(0), :, c0:c0 + 256][None]).reshape(32 * n, 256)
                      for c0 in (l * 256, HALF + l * 256))
            ops = _right_operands(lo[:16 * n], lo[16 * n:], hi[:16 * n], hi[16 * n:])
            for k, op in enumerate(ops):
                h_s[i][k, 8 * b:8 * (b + n), l * 256:(l + 1) * 256] = _bits(op.astype(BF16))

    def layer_norm_rows(i, b, n):
        hold(x_v, tick(NORM_RELEASE))
        row_statistics(i, b, n)
        normalize_rows(i, b, n, (0, 1), back=2)
        return h_s[i][at(0), 8 * b:8 * (b + 1), :128]

    def project(w_s, g, i, tasks):
        blocks = block_product(lambda n: w_s[at(g * NOPS + n)], lambda n: h_s[i][at(n)], tasks)
        return [jnp.concatenate([blocks[j // 2 * 2 + half][j % 2 * 64:(j % 2 + 1) * 64]
                                 for half in range(2)], axis=1) for j in range(4)]

    def features(p, out):
        phi, token = _feature_map(p)
        out.append(phi)
        return token

    def accumulate_kv(v, phi, g, i):
        for j in range(4):
            values = jnp.concatenate([v[j], jnp.ones((16, T), F32)], axis=0).astype(BF16)
            kv = _dot(values, phi[j], _NT)
            kv = kv if i == 0 else kv_acc[j][at(g)] + kv
            if i + 1 < TILES:
                kv_acc[j][g] = kv
            else:
                row = _iota((80, 128), 0)
                head = jnp.where(row < 64, row // DH, row // 8 % 2)
                kv_s[4 * g + j] = _bits(
                    jnp.where(head == _iota((80, 128), 1) % 2, kv, 0.0).astype(BF16))

    wait_all(cp_x[0])
    for b in range(0, 8, 2):
        row_statistics(0, b, 2)
    cp_phi.wait()
    phi_bd = phi_blocks()
    for l in range(2):
        for k in range(4 * l, 4 * l + 4):
            wait_all(cp_mod_a[k])
            modulation(mod_a_cols[k])
        for b in range(0, 8, 2):
            normalize_rows(0, b, 2, (l,))
        if l == 0:
            wait_all(cp_wk[0])
            for k in range(HALF // 128):
                fold_phi(D, wk_s, 0, k)
    wait_all(cp_wv[0])

    def fold_keys(g):
        wait_all(cp_wk[g] + cp_wv[g] + (cp_x[g - 1] if g > 1 else []))
        for l in range(HALF // 128):
            fold_phi(D, wk_s, g, l)

    pending = None
    for u in range(UNITS):
        i, g = divmod(u, GROUPS)
        if LATE_UNIT <= u < LATE_UNIT + 8:
            hold(wqkv_v, tick(13))
            for k in range(2 * (u - LATE_UNIT), 2 * (u - LATE_UNIT + 1)):
                fold_phi(0, wq_s, *divmod(k, HALF // 128))

        if i < 2:
            work = zip(NORM_SLOTS_EARLY, (4 * g - 8, 4 * g - 6), (2, 2), (3, 3)) if g >= 2 else ()
        elif i + 1 < TILES:
            slots = NORM_SLOTS_LATE if u >= LATE_UNIT else NORM_SLOTS
            n = 2 // len(slots)
            work = [(slot, 2 * g + k, n, 2 + n) for k, slot in enumerate(slots)]
        else:
            work = ()
        first, last = split_tasks([(slot, task(layer_norm_rows, i + 1, b, n), slack)
                                   for slot, b, n, slack in work])
        if u == GROUPS + 1:
            first.append((X_WAIT_SLOT, task(wait_all, cp_x[3])))
        if u == LATE_UNIT - 1:
            first.append((LATE_WAIT_SLOT, task(wait_all, cp_late)))
        pk = project(wk_s, g, i, first)
        if i == 0:
            transpose_wv(g)
        if pending is not None:
            accumulate_kv(*pending)
        phi = []
        last += [(KEY_SLOTS[j] - NOPS, task(features, pk[j], phi)) for j in range(4)]
        if u + 1 < GROUPS:
            last.append((KEY_WEIGHT_SLOT - NOPS, task(fold_keys, g + 1)))
        if i == TILES - 1:
            last += [(3 + k, task(transpose_wo, g, k)) for k in range(GROUPS)]
        pending = project(wv_s, g, i, last), phi, g, i
    accumulate_kv(*pending)

    o_parts, o_ops = {}, {}
    no_top = [jnp.full((8, 128), -jnp.inf, F32), jnp.zeros((8, 128), I32)] * 2
    top = list(no_top)

    def output_vectors():
        wr = wr_v[...].astype(F32)
        wr = jnp.concatenate([jnp.broadcast_to(wr[l:l + 1], (8, 128)) for l in range(D // 128)], axis=1)
        shift, scale, gate = mod_b[1], mod_b[2], mod_b[3]
        mod_b[4] = scale * wr
        mod_b[5] = scale * gate
        mod_b[6] = shift * gate
        return _row_sum(shift * wr), _row_sum(scale * wr)

    def attend(phi, g, out):
        out.extend(_dot(_bf16(kv_s[at(4 * g + j)]), phi[j], _NN) for j in range(4))

    def transpose_attention(nums, i, g):
        blocks = []
        for num in nums:
            num = num.reshape(10, 8, T)
            inv = _recip(num[8:] + 1e-6)
            o = jnp.concatenate([num[:4] * inv[0:1], num[4:8] * inv[1:2]], axis=0)
            blocks.append(o.reshape(64, T))
        first = jnp.concatenate(blocks[:2], axis=0).T
        second = jnp.concatenate(blocks[2:], axis=0).T
        quads = first[:128], second[:128], first[128:], second[128:]
        o_parts[i, g] = _left_operands(*quads)
        return _join([_bits(q[120:]) for q in quads])

    def attention_operand(i, n):
        if (i, n) not in o_ops:
            parts = [o_parts[i, g][n] for g in range(GROUPS)]
            o_ops[i, n] = jnp.concatenate(parts, axis=1).astype(BF16)
        return o_ops[i, n]

    def add_residual(blocks, i, cols, order=(2, 1, 0, 3)):
        for k in order:
            hold(x_v, blocks[k][:8])
            cs = pl.ds(cols * 256 + k % 2 * 128, 128)
            x = x_v[pl.ds(at(i * 16 + k // 2 * 8), 8), :, cs].astype(F32).reshape(16, 8, 128)
            x1 = x + mod_b[at(0), :, cs][None] * blocks[k].reshape(16, 8, 128)
            x1_v[i % 2][pl.ds(i // 2 * 16 + k // 2 * 8, 8), :, cs] = x1.reshape(8, 16, 128)
            if i == TILES - 1:
                accumulate_moments(k // 2, x1, cs)

    moments = {}

    def accumulate_moments(half, x1, cs):
        if half not in moments:
            moments[half] = [_row_sum(x1) * (1.0 / 128), None]
        pivot, sums = moments[half]
        d = x1 - pivot
        terms = d, d * d, d * mod_b[at(4), :, cs][None]
        moments[half][1] = terms if sums is None else [s + t for s, t in zip(sums, terms)]

    def load_attended(r0, n):
        i = r0 // T
        return x1_v[i % 2][pl.ds(at(i // 2 * 16 + r0 % T // 16), n // 16)].reshape(n // 8, 8, D)

    def mean_attended(r0, n):
        hold(x1_v[r0 // T % 2], tick(FINISH_RELEASE))
        stats[r0] = _row_sum(load_attended(r0, n)) * (1.0 / D)
        return _join([_bits(jnp.broadcast_to(stats[r0][k], (8, 128))) for k in range(n // 8)])

    def score_rows(r0, n):
        if r0 < S - T:
            mean = stats[r0]
            centered = load_attended(r0, n) - mean
            routed = _row_sum(centered * mod_b[at(4)][None])
            inv = _inv_std(centered)
        else:
            pivot, sums = moments[r0 % T // 128]
            rows = slice(r0 % 128 // 8, (r0 % 128 + n) // 8)
            offset, square, routed = (_row_sum(s[rows]) for s in sums)
            offset = offset * (1.0 / D)
            mean = pivot[rows] + offset
            inv = lax.rsqrt(jnp.maximum(square * (1.0 / D) - offset * offset, 0.0) + 1e-5)
            routed = routed - offset * route_sum
        for k, stat in enumerate((mean, inv)):
            stat_v[k, pl.ds(r0 // 8, n // 8)] = jnp.broadcast_to(stat, (n // 8, 8, 128))
        stats[r0] = mean, inv
        score = _round_bf16(routed * inv + score_bias)
        if S - T <= r0 < S - LAST_ROWS:
            top.extend(no_top)
        best, best_i, second, second_i = top[-4:]
        for b in range(n // 8):
            s, t = jnp.broadcast_to(score[b], (8, 128)), _iota((8, 128), 0) + (r0 + 8 * b)
            above_best, above_second = s > best, s > second
            second = jnp.where(above_best, best, jnp.where(above_second, s, second))
            second_i = jnp.where(above_best, best_i, jnp.where(above_second, t, second_i))
            best = jnp.where(above_best, s, best)
            best_i = jnp.where(above_best, t, best_i)
        top[-4:] = best, best_i, second, second_i

    def output_rows(r0, n, token=None):
        mean, inv = stats[r0]
        if token is not None:
            inv = once(inv, token[None])
        x1 = load_attended(r0, n)
        out = x1 + ((x1 - once(mean, inv)) * inv * mod_b[at(5)][None] + mod_b[at(6)][None])
        out_v[pl.ds(r0 // 16, n // 16)] = out.reshape(n // 16, 16, D).astype(BF16)

    def finish_rows(r0, n):
        score_rows(r0, n)
        output_rows(r0, n)
        return _bits(top[3]) | _bits(out_v[at(0), :, :128])

    phi = attn = None
    finished = 0
    for u in range(UNITS + LAG):
        tasks = []
        if phi is not None:
            nums = []
            slots = ATTEND_SLOTS if u < UNITS else ATTEND_SLOTS_LAST
            tasks += [(slots[0], task(attend, phi, (u - 1) % GROUPS, nums)),
                      (slots[1], task(transpose_attention, nums, *divmod(u - 1, GROUPS)), 1)]
        if attn is not None:
            add_residual(attn, *divmod(u - LAG - 1, GROUPS))
        if u >= LAG + GROUPS:
            n = 32 if u < UNITS + LAG - GROUPS else FINISH_ROWS_LAST[u - UNITS - LAG]
            for slots in (FINISH_SLOTS if u < UNITS else FINISH_SLOTS_LAST) if n else ():
                tasks += [(slots[0], task(mean_attended, finished, n)),
                          (slots[1], task(finish_rows, finished, n), 1)]
                finished += n
        if u == (EARLY_TILES + 1) * GROUPS + LAG:
            tasks.append((OUTPUT_SLOT, cp_out[0].start))
        first, last = split_tasks(tasks)
        phi = None
        if u < UNITS:
            pq, phi = project(wq_s, u % GROUPS, u // GROUPS, first), []
            last += [(QUERY_SLOTS[j] - NOPS, task(features, pq[j], phi)) for j in range(4)]
        if u >= LAG:
            i, cols = divmod(u - LAG, GROUPS)
            attn = block_product(task(attention_operand, i), lambda n: wo_s[at(cols * NOPS + n)], last,
                                 lower_first=u + 1 == UNITS + LAG)
        else:
            for _, fn in last:
                fn()
            for k in range(16 * u // LAG, 16 * (u + 1) // LAG):
                modulation(2 * D + 256 * k)
            if u == LAG - 1:
                score_bias, route_sum = output_vectors()
    add_residual(attn, TILES - 1, GROUPS - 1, order=(2, 3, 1, 0))
    assert finished == S - T
    for r0 in reversed(range(S - T, S, LAST_ROWS)):
        score_rows(r0, LAST_ROWS)

    scores = jnp.concatenate(top[0::2], axis=0)
    tokens = jnp.concatenate(top[1::2], axis=0)

    def take_top(scores):
        score = jnp.max(scores, axis=0, keepdims=True)
        token = jnp.min(jnp.where(scores == score, tokens, S - 1).astype(F32), axis=0, keepdims=True)
        return score, token.astype(I32)

    score0, token0 = take_top(scores)
    score1, token1 = take_top(jnp.where(tokens == token0, -jnp.inf, scores))
    cp_out[1].start()
    wait_all(cp_ffn)
    routed = [jnp.clip(token[0, 0], 0, S - 1) for token in (token0, token1)]

    row16 = _iota((16, D), 0)
    shift, scale, gate_b = mod_b[at(1)], mod_b[at(2)], mod_b[at(3)]
    x1_sel = h2_sel = weight = jnp.zeros((16, D), F32)
    for k, (t, score) in enumerate(zip(routed, (score0, score1))):
        blk, row = t // (2 * T) * 16 + t % T // 16, pl.ds(t % 16, 1)
        x1 = jnp.where(t // T % 2 == 0, x1_v[0][blk, row, :], x1_v[1][blk, row, :])
        mean, inv = (jnp.tile(stat_v[m, t // 8, pl.ds(t % 8, 1), :], (1, D // 128)) for m in range(2))
        x1_sel = jnp.where(row16 == k, x1, x1_sel)
        h2_sel = jnp.where(row16 == k, (x1 - mean) * inv * scale[:1] + shift[:1], h2_sel)
        weight = jnp.where(row16 == k, jnp.tile(jax.nn.sigmoid(score), (1, D // 128)), weight)
    h_sel = h2_sel.astype(BF16)
    gate_b = jnp.concatenate([gate_b, gate_b], axis=0)
    base_rows, update_scale = x1_sel + gate_b * h2_sel, gate_b * weight

    def down(f, act):
        return _dot(act, wd_v[f * F_CHUNK:(f + 1) * F_CHUNK, :], _NN)

    y, act = jnp.zeros((16, D), F32), None
    for f in range(F // F_CHUNK):
        gate, up = (_dot(h_sel, w[:, f * F_CHUNK:(f + 1) * F_CHUNK], _NN) for w in (wg_v, wu_v))
        if f > 0:
            y = y + down(f - 1, act)
        act = (gate * jax.nn.sigmoid(gate) * up).astype(BF16)
        if f < T // LAST_ROWS:
            output_rows(S - T + f * LAST_ROWS, LAST_ROWS, gate[:8, :1])
        if f == T // LAST_ROWS:
            cp_out[2].start()
    routed_rows = base_rows + update_scale * (y + down(F // F_CHUNK - 1, act))

    wait_all(cp_out)
    for k, t in enumerate(routed):
        row = jnp.broadcast_to(routed_rows[k:k + 1], (16, D))
        out_v[t // 16] = jnp.where(row16 == t % 16, row, out_v[t // 16].astype(F32)).astype(BF16)
    fix = [copy(out_v.at[t // 16], out_hbm.at[t // 16]) for t in routed]
    fix[0].start()

    @pl.when(routed[0] // 16 != routed[1] // 16)
    def _():
        fix[1].start()
        fix[1].wait()

    fix[0].wait()


@jax.jit
def pallas_adaLN_cond__linear_kernel_hedgehog__moe_arch_mod__prompt_kernel(
    A_x: jax.Array,
    A_wqkv: jax.Array,
    A_w_phi: jax.Array,
    A_wo: jax.Array,
    B_x: jax.Array,
    B_w_r: jax.Array,
    B_w_gate: jax.Array,
    B_w_up: jax.Array,
    B_w_down: jax.Array,
    c: jax.Array,
    w_mod: jax.Array,
):
    del B_x
    weight_operands = pltpu.VMEM((GROUPS * NOPS, 64, HALF), U32)
    out = pl.pallas_call(
        _kernel,
        out_shape=jax.ShapeDtypeStruct((S // 16, 16, D), BF16),
        in_specs=[pl.BlockSpec(memory_space=pl.ANY)] * 10,
        out_specs=pl.BlockSpec(memory_space=pl.ANY),
        scratch_shapes=[
            pltpu.VMEM((S // 16 + 1, 16, D), BF16),
            pltpu.VMEM((3 * D // 128 + 1, D, 128), BF16),
            pltpu.VMEM((H * DH, DH), BF16),
            pltpu.VMEM((GROUPS + 1, 256, D), BF16),
            pltpu.VMEM((D // 128, 128), BF16),
            pltpu.VMEM((D, F), BF16),
            pltpu.VMEM((D, F), BF16),
            pltpu.VMEM((F, D), BF16),
            pltpu.VMEM((1, D), BF16),
            pltpu.VMEM((6 * D // 128, D, 128), BF16),
            weight_operands,
            weight_operands,
            weight_operands,
            weight_operands,
            pltpu.VMEM((S // 16, 16, D), BF16),
            pltpu.VMEM((2, 8, D), F32),
            pltpu.VMEM((7, 8, D), F32),
            pltpu.VMEM((H // 2, 40, 128), U32),
            pltpu.VMEM((2, S // 8, 8, 128), F32),
            pltpu.SemaphoreType.DMA((40,)),
            *[pltpu.VMEM((S // 32 + 1, 16, D), F32)] * 2,
            *[pltpu.VMEM((GROUPS, 80, 128), F32)] * 4,
            *[pltpu.VMEM((NOPS, 64, HALF), U32)] * TILES,
        ],
        compiler_params=pltpu.CompilerParams(vmem_limit_bytes=120 * 1024 * 1024),
        name="hedgehog_moe",
    )(
        A_x.reshape(S // 16, 16, D), A_wqkv, A_w_phi.reshape(H * DH, DH),
        A_wo.reshape(GROUPS, 256, D), B_w_r.reshape(D // 128, 128),
        B_w_gate, B_w_up, B_w_down, c, w_mod,
    )
    return out.reshape(1, S, D)
```
